```python
import jax
import jax.numpy as jnp

def _softmax(x, axis=-1):
    return jax.nn.softmax(x, axis=axis)
def _gelu(x):
    return jax.nn.gelu(x, approximate=True)
def _silu(x):
    return jax.nn.silu(x)
def _sigmoid(x):
    return jax.nn.sigmoid(x)
def _layernorm(x, axis=-1, eps=1e-5):
    m = jnp.mean(x, axis=axis, keepdims=True)
    v = jnp.var(x, axis=axis, keepdims=True)
    return (x - m) / jnp.sqrt(v + eps)
def _scatter_add(tgt, idx, src, axis=0):
    return tgt.at[idx].add(src)
def _segment_sum(src, seg, n):
    return jax.ops.segment_sum(src, seg, n)
class _Rng:
    def __init__(self, key):
        self._k = key
    def _next(self):
        self._k, sub = jax.random.split(self._k)
        return sub
    def normal(self, shape):
        return jax.random.normal(self._next(), shape, dtype=jnp.bfloat16)
    def randint(self, lo, hi, shape):
        return jax.random.randint(self._next(), shape, lo, hi, dtype=jnp.int32)
    def uniform(self, shape, lo=0.0, hi=1.0):
        return jax.random.uniform(self._next(), shape, jnp.bfloat16, lo, hi)
    def permutation(self, n):
        return jax.random.permutation(self._next(), n)


kernel_name = 'interleave_layers__sliding_block_cached__mixer_s_mlp__decode'

def setup_inputs():
    _rng = _Rng(jax.random.key(int.from_bytes(__import__("os").urandom(4), "little")))
    _w = (lambda a: (lambda t: t.astype(jnp.bfloat16) if jnp.issubdtype(t.dtype, jnp.floating) else t)(jnp.asarray(a)))
    def _A_setup():
        B, Sq, D = 1, 1, 640
        Hq, Hkv, Sk, Dh = 32, 32, 32768, 192
        assert Hq % Hkv == 0, (Hq, Hkv)
        return {
            "x": _w((lambda *s: _rng.normal(s) * 0.05)(B, Sq, D)),
            "k_cache": _w((lambda *s: _rng.normal(s) * 0.05)(B, Hkv, Sk, Dh)),
            "v_cache": _w((lambda *s: _rng.normal(s) * 0.05)(B, Hkv, Sk, Dh)),
            "wq": _w((lambda *s: _rng.normal(s) * 0.05)(D, Hq * Dh) * (D ** -0.5)),
            "wo": _w((lambda *s: _rng.normal(s) * 0.05)(Hq * Dh, D) * ((Hq * Dh) ** -0.5)),
        }
    _A_in = _A_setup()

    def _B_setup():
        B, S, D, F = 1, 1, 640, 1536
        return {
            "x":  _w((lambda *s: _rng.normal(s) * 0.05)(B, S, D)),
            "w1": _w((lambda *s: _rng.normal(s) * 0.05)(D, D) * (D ** -0.5)),
            "w2": _w((lambda *s: _rng.normal(s) * 0.05)(D, D) * (D ** -0.5)),
            "w3": _w((lambda *s: _rng.normal(s) * 0.05)(D, F) * (D ** -0.5)),
            "w4": _w((lambda *s: _rng.normal(s) * 0.05)(F, D) * (F ** -0.5)),
        }
    _B_in = _B_setup()

    return {
        "A_x": _A_in["x"],
        "A_k_cache": _A_in["k_cache"],
        "A_v_cache": _A_in["v_cache"],
        "A_wq": _A_in["wq"],
        "A_wo": _A_in["wo"],
        "B_x": _B_in["x"],
        "B_w1": _B_in["w1"],
        "B_w2": _B_in["w2"],
        "B_w3": _B_in["w3"],
        "B_w4": _B_in["w4"],
    }

def reference(A_x, A_k_cache, A_v_cache, A_wq, A_wo, B_x, B_w1, B_w2, B_w3, B_w4):
    def _A_ref(x, k_cache, v_cache, wq, wo):
        B, Sq, D = x.shape
        Hq, Dh = 32, 192
        Hkv, Sk = k_cache.shape[1], k_cache.shape[2]
        W = min(4096, max(256, Sk // 4))
        rep = Hq // Hkv
        q = (lambda x, *d: x.transpose(*d))((x @ wq).reshape(B, Sq, Hq, Dh), 0, 2, 1, 3)
        k = jnp.repeat(k_cache[:, :, Sk - W:, :], rep, axis=1)
        v = jnp.repeat(v_cache[:, :, Sk - W:, :], rep, axis=1)
        scores = jnp.einsum("bhqd,bhkd->bhqk", q, k) * (Dh ** -0.5)
        p = _softmax(scores, axis=-1)
        o = jnp.einsum("bhqk,bhkd->bhqd", p, v)
        return (lambda x, *d: x.transpose(*d))(o, 0, 2, 1, 3).reshape(B, Sq, Hq * Dh) @ wo

    def _B_ref(x, w1, w2, w3, w4):
        B, S, D = x.shape
        h = _gelu(_layernorm(x, axis=-1) @ w1)
        c = D // 4
        g0 = jnp.pad(h[:, :, 0*c:1*c], ((0, 0), (1, 0), (0, 0)))[:, :S, :]
        g1 = jnp.pad(h[:, :, 1*c:2*c], ((0, 0), (0, 1), (0, 0)))[:, 1:, :]
        g2 = jnp.pad(h[:, :, 2*c:3*c], ((0, 0), (2, 0), (0, 0)))[:, :S, :]
        g3 = jnp.pad(h[:, :, 3*c:   ], ((0, 0), (0, 2), (0, 0)))[:, 2:, :]
        hs = jnp.concatenate([g0, g1, g2, g3], axis=-1) @ w2
        x1 = x + hs
        h2 = _gelu(_layernorm(x1, axis=-1) @ w3) @ w4
        return x1 + h2

    x = A_x
    x = x + _A_ref(_layernorm(x, axis=-1), A_k_cache, A_v_cache, A_wq, A_wo)
    x = x + _B_ref(_layernorm(x, axis=-1), B_w1, B_w2, B_w3, B_w4)
    x = x + _A_ref(_layernorm(x, axis=-1), A_k_cache, A_v_cache, A_wq, A_wo)
    x = x + _B_ref(_layernorm(x, axis=-1), B_w1, B_w2, B_w3, B_w4)
    return x
```

```python
import functools
import jax
import jax.numpy as jnp
from jax import lax
import jax.experimental.pallas as pl
import jax.experimental.pallas.tpu as pltpu

D = 640
H = 32
DH = 192
F = 1536
NP = H // 2
PD = 2 * DH
LOG2E = 1.4426950408889634
EPS = 1e-5
BF = jnp.bfloat16
F32 = jnp.float32


def _ln(x):
    m = jnp.mean(x, axis=-1, keepdims=True)
    c = x - m
    v = jnp.mean(c * c, axis=-1, keepdims=True)
    return c * lax.rsqrt(v + EPS)


def _bf(w):
    return pltpu.bitcast(w, BF)


FLAGS = None
def build(SK, W, DEPTH=3, NACC=12, ORDER=0):
    S0 = SK - W
    NT = W // 128
    QSCALE = (DH ** -0.5) * LOG2E

    def kernel(x_hbm, k_hbm, v_hbm, wq_hbm, wo_hbm, w3_hbm, w4_hbm, o_hbm,
               kbuf, vbuf, wqb, wob, w3b, w4b, pbufa, pbufb, xbuf, obuf, ksem, vsem, wsem):
        pbufs = (pbufa, pbufb)
        k32 = k_hbm.bitcast(jnp.uint32)
        v32 = v_hbm.bitcast(jnp.uint32)

        def kcp(j):
            return pltpu.make_async_copy(k32.at[pl.ds(2 * j, 2), :, pl.ds(S0, W)], kbuf.at[pl.ds(2 * j, 2)], ksem.at[j])

        def vcp(j):
            return pltpu.make_async_copy(v32.at[pl.ds(2 * j, 2), :, pl.ds(S0, W)], vbuf.at[pl.ds(2 * j, 2)], vsem.at[j])

        wq_cp = pltpu.make_async_copy(wq_hbm.bitcast(jnp.uint32), wqb, wsem.at[0])
        wo_cp = pltpu.make_async_copy(wo_hbm.bitcast(jnp.uint32), wob, wsem.at[1])
        w3_cp = pltpu.make_async_copy(w3_hbm.bitcast(jnp.uint32), w3b, wsem.at[2])
        w4_cp = pltpu.make_async_copy(w4_hbm.bitcast(jnp.uint32), w4b, wsem.at[3])
        x_cp = pltpu.make_async_copy(x_hbm, xbuf, wsem.at[4])
        o_cp = pltpu.make_async_copy(obuf, o_hbm, wsem.at[5])

        wq_cp.start()
        x_cp.start()
        kcp(0).start()
        wo_cp.start()
        def issue(i):
            if i + 1 < NP:
                kcp(i + 1).start()
            vcp(i).start()
            if i == NP - 1:
                w3_cp.start()
                w4_cp.start()
        for i in range(DEPTH):
            issue(i)

        lane = lax.broadcasted_iota(jnp.int32, (8, PD), 1)
        in_a = lane < DH

        def qproj(xl, j):
            w = _bf(wqb[:, pl.ds(pl.multiple_of(j * PD, 128), PD)])
            q = jnp.dot(xl, w, preferred_element_type=F32) * QSCALE
            qa = jnp.where(in_a, q, 0.0)
            qb = jnp.where(in_a, 0.0, q)
            return jnp.concatenate([qa, qb], axis=0).astype(BF)

        def qk(ql, j, slot):
            k = _bf(kbuf[pl.ds(2 * j, 2)].reshape(PD // 2, W))
            s = jnp.dot(ql, k, preferred_element_type=F32)
            m = jnp.max(s, axis=1, keepdims=True)
            e = jnp.exp2(s - m)
            pbufs[slot][...] = e
            l = jnp.sum(e, axis=1, keepdims=True)
            inv = 1.0 / l
            inv = jnp.broadcast_to(inv, (16, 128))
            ia = jnp.concatenate([inv[0:8]] * 3, axis=1)
            ib = jnp.concatenate([inv[8:16]] * 3, axis=1)
            return jnp.where(in_a, ia, ib)

        def pv(j, slot, inv):
            accs = []
            for hh in range(2):
                for g in range(12 // NACC):
                    acc = [jnp.zeros((16, 128), F32) for _ in range(NACC)]
                    for t in range(NT):
                        pb = pbufs[slot][hh * 8:(hh + 1) * 8, t * 128:(t + 1) * 128]
                        pb = jnp.concatenate([pb, pb], axis=0)
                        for i in range(NACC):
                            r0 = (g * NACC + i) * 8
                            w = vbuf[2 * j + hh, r0:r0 + 8, t * 128:(t + 1) * 128]
                            acc[i] = acc[i] + _bf(w).astype(F32) * pb
                    accs.extend(acc)
            a = jnp.concatenate(accs, axis=0)
            o = jnp.sum(a.T, axis=0, keepdims=True)
            o = jnp.broadcast_to(o, (8, PD)) * inv
            return o.astype(BF)

        def wo_dot(o, j):
            w = _bf(wob[pl.ds(pl.multiple_of(j * (PD // 2), 8), PD // 2), :])
            return jnp.dot(o, w, preferred_element_type=F32)

        def attention(x, first):
            xl = _ln(x).astype(BF)
            if first:
                wq_cp.wait()
            q0 = qproj(xl, 0)
            q1 = qproj(xl, 1)
            if first:
                kcp(0).wait()
                wo_cp.wait()
            inv0 = qk(q0, 0, 0)

            def step(j, slot, carry):
                qn, inv, o_prev, acc = carry
                if first:
                    @pl.when(j + 1 < NP)
                    def _():
                        kcp(j + 1).wait()
                    vcp(j).wait()
                    @pl.when(j + DEPTH < NP)
                    def _():
                        i = j + DEPTH
                        @pl.when(i + 1 < NP)
                        def _():
                            kcp(i + 1).start()
                        vcp(i).start()
                        @pl.when(i == NP - 1)
                        def _():
                            w3_cp.start()
                            w4_cp.start()
                jn = jnp.minimum(j + 1, NP - 1)
                jnn = jnp.minimum(j + 2, NP - 1)
                jp = jnp.maximum(j - 1, 0)
                if ORDER == 0:
                    acc = acc + wo_dot(o_prev, jp)
                    q2 = qproj(xl, jnn)
                    inv_n = qk(qn, jn, 1 - slot)
                    o = pv(j, slot, inv)
                else:
                    o = pv(j, slot, inv)
                    inv_n = qk(qn, jn, 1 - slot)
                    acc = acc + wo_dot(o_prev, jp)
                    q2 = qproj(xl, jnn)
                return q2, inv_n, o, acc

            def body(jj, carry):
                carry = step(2 * jj, 0, carry)
                return step(2 * jj + 1, 1, carry)

            _, _, o_last, acc = lax.fori_loop(
                0, NP // 2, body, (q1, inv0, jnp.zeros((8, PD), BF), jnp.zeros((8, D), F32)))
            return x + acc + wo_dot(o_last, NP - 1)

        def mlp(x, first):
            u = _ln(x)
            h = _ln(u).astype(BF)
            if first:
                w3_cp.wait()
            g = jnp.dot(h, _bf(w3b[...]), preferred_element_type=F32)
            g = jax.nn.gelu(g, approximate=True).astype(BF)
            if first:
                w4_cp.wait()
            return x + u + jnp.dot(g, _bf(w4b[...]), preferred_element_type=F32)

        x_cp.wait()
        x = jnp.broadcast_to(xbuf[0].astype(F32), (8, D))
        x = attention(x, True)
        x = mlp(x, True)
        x = attention(x, False)
        x = mlp(x, False)
        obuf[0] = x[0:1].astype(BF)
        o_cp.start()
        o_cp.wait()

    def fn(A_x, A_k_cache, A_v_cache, A_wq, A_wo, B_x, B_w1, B_w2, B_w3, B_w4):
        kT = jnp.swapaxes(A_k_cache[0], 1, 2)
        vT = jnp.swapaxes(A_v_cache[0], 1, 2)
        return pl.pallas_call(
            kernel,
            out_shape=jax.ShapeDtypeStruct((1, 1, D), BF),
            in_specs=[pl.BlockSpec(memory_space=pl.ANY)] * 7,
            out_specs=pl.BlockSpec(memory_space=pl.ANY),
            scratch_shapes=[
                pltpu.VMEM((H, DH // 2, W), jnp.uint32),
                pltpu.VMEM((H, DH // 2, W), jnp.uint32),
                pltpu.VMEM((D // 2, H * DH), jnp.uint32),
                pltpu.VMEM((H * DH // 2, D), jnp.uint32),
                pltpu.VMEM((D // 2, F), jnp.uint32),
                pltpu.VMEM((F // 2, D), jnp.uint32),
                pltpu.VMEM((16, W), F32),
                pltpu.VMEM((16, W), F32),
                pltpu.VMEM((1, 1, D), BF),
                pltpu.VMEM((1, 1, D), BF),
                pltpu.SemaphoreType.DMA((NP,)),
                pltpu.SemaphoreType.DMA((NP,)),
                pltpu.SemaphoreType.DMA((6,)),
            ],
            compiler_params=pltpu.CompilerParams(vmem_limit_bytes=127 * 2**20, flags=FLAGS),
        )(A_x, kT, vT, A_wq, A_wo, B_w3, B_w4)
    return fn


@jax.jit
def pallas_interleave_layers__sliding_block_cached__mixer_s_mlp__decode_kernel(
    A_x: jax.Array,
    A_k_cache: jax.Array,
    A_v_cache: jax.Array,
    A_wq: jax.Array,
    A_wo: jax.Array,
    B_x: jax.Array,
    B_w1: jax.Array,
    B_w2: jax.Array,
    B_w3: jax.Array,
    B_w4: jax.Array,
):
    sk = A_k_cache.shape[2]
    w = min(4096, max(256, sk // 4))
    return build(sk, w, ORDER=1)(A_x, A_k_cache, A_v_cache, A_wq, A_wo, B_x, B_w1, B_w2, B_w3, B_w4)
```

```python
import jax
import jax.numpy as jnp
from jax import lax
import jax.experimental.pallas as pl
import jax.experimental.pallas.tpu as pltpu

D = 640
H = 32
DH = 192
F = 1536
NP = H // 2
PD = 2 * DH
LOG2E = 1.4426950408889634
EPS = 1e-5
BF = jnp.bfloat16
F32 = jnp.float32
U32 = jnp.uint32


def _ln(x):
    m = jnp.mean(x, axis=-1, keepdims=True)
    c = x - m
    v = jnp.mean(c * c, axis=-1, keepdims=True)
    return c * lax.rsqrt(v + EPS)


def _bf(w):
    return pltpu.bitcast(w, BF)


def _u(x):
    return pltpu.bitcast(x, U32)


def _raw2(a):
    *lead, r, c = a.shape
    n = len(lead)
    z = a.reshape(*lead, r // 8, 8, c // 256, 2, 128)
    z = z.transpose(*range(n), n, n + 2, n + 3, n + 1, n + 4)
    return z.reshape(*lead, r // 8, c // 256, 16, 128)


def _raw5(a):
    r, c = a.shape
    z = a.reshape(r // 8, 8, 5, 128).transpose(0, 2, 1, 3)
    return z.reshape(r // 16, 5, 16, 128)


FLAGS = None
def build(SK, W, DEPTH=4, REP=1, NA=2, QA=1, QB=10, QAE=1, QBE=10, EG=6, EGS=2, FG=8, XK=8, W4C=4):
    NCP = W // 256
    CP0 = (SK - W) // 256
    QSCALE = (DH ** -0.5) * LOG2E
    groups = [NA] * (24 // NA)
    NG = len(groups)

    def kernel(x_hbm, k_hbm, v_hbm, wq_hbm, wo_hbm, w3_hbm, w4_hbm, o_hbm,
               kb, vb, wqb, wob, w3b, w4b, eca, sa, sb, ea, eb, mxa, mxb, accb, lb, Lb, xab, ob, xlb,
               xbuf, obuf, ksem, vsem, wsem):
        k32 = k_hbm.bitcast(U32)
        v32 = v_hbm.bitcast(U32)

        def kcp(h):
            return pltpu.make_async_copy(k32.at[h, :, pl.ds(CP0, NCP)], kb.at[h], ksem.at[h])

        def vcp(h):
            return pltpu.make_async_copy(v32.at[h, :, pl.ds(CP0, NCP)], vb.at[h], vsem.at[h])

        wq_cp = pltpu.make_async_copy(wq_hbm.bitcast(U32), wqb, wsem.at[0])
        wo_cp = pltpu.make_async_copy(wo_hbm.bitcast(U32), wob, wsem.at[1])
        w3_cp = pltpu.make_async_copy(w3_hbm.bitcast(U32), w3b, wsem.at[2])
        x_cp = pltpu.make_async_copy(x_hbm, xbuf, wsem.at[3])
        o_cp = pltpu.make_async_copy(obuf, o_hbm, wsem.at[4])
        R4 = F // 2 // W4C
        w4_cp = [pltpu.make_async_copy(w4_hbm.bitcast(U32).at[pl.ds(i * R4, R4)], w4b.at[pl.ds(i * R4, R4)], wsem.at[5 + i])
                 for i in range(W4C)]

        def issue_static(i):
            if i + 2 < H:
                kcp(i + 2).start()
            vcp(i).start()

        wq_cp.start()
        x_cp.start()
        kcp(0).start()
        kcp(1).start()
        wo_cp.start()
        for i in range(DEPTH):
            issue_static(i)

        low = lax.broadcasted_iota(jnp.int32, (8, 128), 0) < 4
        in_a = lax.broadcasted_iota(jnp.int32, (8, PD), 1) < DH

        def make_expand_matrix():
            row = lax.broadcasted_iota(jnp.int32, (128, 512), 0)
            col = lax.broadcasted_iota(jnp.int32, (128, 512), 1)
            hi = row >> 6
            jj = row & 63
            u = col >> 7
            cond = ((u >> 1) == hi) & ((col & 127) == ((jj >> 3) << 4) + ((u & 1) << 3) + (jj & 7))
            eca[...] = jnp.where(cond, 1.0, 0.0).astype(BF)

        def retile_wq():
            def body(g, _):
                for c in range(24):
                    a = wqb[2 * g, c]
                    b = wqb[2 * g + 1, c]
                    wqb[2 * g, c] = jnp.where(low, a, pltpu.roll(b, 4, 0))
                    wqb[2 * g + 1, c] = jnp.where(low, pltpu.roll(a, 4, 0), b)
                return _
            lax.fori_loop(0, 40, body, 0)

        def retile_wo():
            def body(gg, _):
                for u in range(4):
                    g = gg * 4 + u
                    raw = [wob[g, p] for p in range(5)]
                    rot = [pltpu.roll(r, 4, 0) for r in raw]
                    for c in range(5):
                        t1, t2 = c, 5 + c
                        top = raw[t1 // 2] if t1 % 2 == 0 else rot[t1 // 2]
                        bot = rot[t2 // 2] if t2 % 2 == 0 else raw[t2 // 2]
                        wob[g, c] = jnp.where(low, top, bot)
                return _
            lax.fori_loop(0, 96, body, 0)

        def qproj(p):
            cols = []
            for u in range(3):
                t = 3 * p + u
                w = wqb[pl.ds(t % 2, 40, stride=2), t // 2]
                cols.append(_bf(w.reshape(320, 128)))
            return jnp.dot(xlb[...], jnp.concatenate(cols, axis=1), preferred_element_type=F32)

        def expand(q):
            q = (q * QSCALE).astype(BF)
            qs = jnp.concatenate([q[:, 0:128], q[:, 128:256], q[:, 256:384]], axis=0)
            ex = jnp.dot(qs, eca[...], preferred_element_type=F32)

            def tile(t, hi):
                return jnp.concatenate([ex[t * 8:(t + 1) * 8, (2 * hi) * 128:(2 * hi + 1) * 128],
                                        ex[t * 8:(t + 1) * 8, (2 * hi + 1) * 128:(2 * hi + 2) * 128]], axis=0)
            la = jnp.concatenate([tile(0, 0), tile(0, 1), tile(1, 0)], axis=1).astype(BF)
            lb_ = jnp.concatenate([tile(1, 1), tile(2, 0), tile(2, 1)], axis=1).astype(BF)
            return la, lb_

        def qk(h, L, dst, mxd, gates=None, z=None, cb=None, qa=0, qb=0):
            ms = []
            for c in range(NCP):
                w = kb[h, :, c]
                if gates is not None:
                    gi = min(qa + ((qb - qa) * c) // NCP, NG - 1)
                    fz = _u(gates[gi]) & z
                    w = jnp.concatenate([w[r] | fz if r == 23 else w[r] for r in range(24)], axis=0)
                else:
                    w = w.reshape(192, 128)
                s = jnp.dot(L, _bf(w), preferred_element_type=F32)
                dst[:, c * 128:(c + 1) * 128] = s
                ms.append(s)
                if cb is not None and c == XK:
                    cb()
            m = ms[0]
            for t in ms[1:]:
                m = jnp.maximum(m, t)
            mxd[...] = jnp.maximum(m[0:8], m[8:16])

        def expo(src, mxs, edst):
            mh = jnp.broadcast_to(jnp.max(mxs[...], axis=1, keepdims=True), (8, 128))
            parts = []
            for c in range(NCP):
                e0 = jnp.exp2(src[0:8, c * 128:(c + 1) * 128] - mh)
                e1 = jnp.exp2(src[8:16, c * 128:(c + 1) * 128] - mh)
                edst[0:8, c * 128:(c + 1) * 128] = e0
                edst[8:16, c * 128:(c + 1) * 128] = e1
                parts.append(e1)
            return parts

        def pv(h, esrc, par, eparts, pre, z):
            r0 = 0
            outs = []
            prev = None
            l = jnp.zeros((8, 128), F32)
            for gi, na in enumerate(groups):
                deps = []
                if prev is not None:
                    deps.append(prev[0])
                if EG <= gi < EG + EGS:
                    k0 = ((gi - EG) * NCP) // EGS
                    k1 = ((gi - EG + 1) * NCP) // EGS
                    for k in range(k0, k1):
                        if (k - k0) % 2 == 1 or k == k1 - 1:
                            deps.append(eparts[k])
                for pg, val in pre:
                    if pg == gi:
                        deps.append(val)
                if deps:
                    t = _u(deps[0])
                    for dd in deps[1:]:
                        t = t | _u(dd)
                    acc0 = pltpu.bitcast(t & z, F32)
                else:
                    acc0 = jnp.zeros((8, 128), F32)
                acc = [acc0 for _ in range(na)]
                for c in range(NCP):
                    e0 = esrc[0:8, c * 128:(c + 1) * 128]
                    e1 = esrc[8:16, c * 128:(c + 1) * 128]
                    if gi == 0:
                        l = l + (e0 + e1)
                    for r in range(na):
                        f = _bf(vb[h, r0 + r, c]).astype(F32)
                        acc[r] = acc[r] + (f[0:8] * e0 + f[8:16] * e1)
                for r in range(na):
                    accb[par * 192 + (r0 + r) * 8: par * 192 + (r0 + r) * 8 + 8, :] = acc[r]
                r0 += na
                prev = acc
                outs.append(acc[0])
            lb[par * 8:(par + 1) * 8, :] = l
            return outs

        def finish():
            o = jnp.sum(accb[...].T, axis=0, keepdims=True)
            inv = 1.0 / jnp.sum(lb[...], axis=1, keepdims=True)
            o = jnp.broadcast_to(o, (8, PD)) * jnp.where(in_a, inv[0:8], inv[8:16])
            return o

        def wo_dot(o, p):
            g0 = pl.multiple_of(p * 24, 8)
            cols = [_bf(wob[pl.ds(g0, 24), c].reshape(192, 128)) for c in range(5)]
            return jnp.dot(o.astype(BF), jnp.concatenate(cols, axis=1), preferred_element_type=F32)

        def step(h, par, s_src, s_dst, e_src, e_dst, mx_src, mx_dst):
            z = jnp.broadcast_to(lax.shift_right_arithmetic(h, 31), (8, 128)).astype(U32)
            hn = jnp.minimum(h + 2, H - 1)
            p = h // 2
            L = Lb[(hn // 2) % 2, par]
            pre = []
            cb = None
            if par == 0:
                pn = jnp.minimum(p + 2, NP - 1)
                q = qproj(pn)

                def cb():
                    la, lb_ = expand(q)
                    Lb[pn % 2, 0] = la
                    Lb[pn % 2, 1] = lb_
                o = finish()
                ob[...] = o
                if FG:
                    pre.append((FG, o[:, 0:128]))
            else:
                xab[...] += wo_dot(ob[...], jnp.maximum(p - 1, 0))
            eparts = expo(s_src, mx_src, e_dst)
            gates = pv(h, e_src, par, eparts, pre, z)
            qk(hn, L, s_dst, mx_dst, gates, z, cb, QAE if par == 0 else QA, QBE if par == 0 else QB)

        def attention(x, first):
            xlb[...] = _ln(x).astype(BF)
            if first:
                make_expand_matrix()
                wq_cp.wait()
                retile_wq()
            la, lb_ = expand(qproj(0))
            la1, lb1 = expand(qproj(1))
            Lb[1, 0] = la1
            Lb[1, 1] = lb1
            if first:
                kcp(0).wait()
                kcp(1).wait()
            qk(0, la, sb, mxb)
            qk(1, lb_, sa, mxa)
            expo(sb, mxb, ea)
            xab[...] = jnp.zeros_like(xab)
            accb[...] = jnp.zeros_like(accb)
            lb[...] = jnp.ones_like(lb)
            if first:
                wo_cp.wait()
                retile_wo()

            def body(h, carry):
                if first:
                    @pl.when(h + 2 < H)
                    def _():
                        kcp(h + 2).wait()
                    vcp(h).wait()

                    @pl.when(h + DEPTH < H)
                    def _():
                        i = h + DEPTH

                        @pl.when(i + 2 < H)
                        def _():
                            kcp(i + 2).start()
                        vcp(i).start()

                        @pl.when(i == H - 1)
                        def _():
                            w3_cp.start()
                            for c in w4_cp:
                                c.start()

                @pl.when(h % 2 == 0)
                def _():
                    step(h, 0, sa, sb, ea, eb, mxa, mxb)

                @pl.when(h % 2 == 1)
                def _():
                    step(h, 1, sb, sa, eb, ea, mxb, mxa)
                return carry

            lax.fori_loop(0, H, body, 0)
            return x + xab[...] + wo_dot(finish(), NP - 1)

        def mlp(x, first):
            u = _ln(x)
            h = _ln(u).astype(BF)
            if first:
                w3_cp.wait()
            g = jnp.dot(h, _bf(w3b[...]), preferred_element_type=F32)
            g = jax.nn.gelu(g, approximate=True).astype(BF)
            y = x + u
            if first:
                for i in range(W4C):
                    w4_cp[i].wait()
                    y = y + jnp.dot(g[:, i * 2 * R4:(i + 1) * 2 * R4], _bf(w4b[i * R4:(i + 1) * R4, :]), preferred_element_type=F32)
            else:
                y = y + jnp.dot(g, _bf(w4b[...]), preferred_element_type=F32)
            return y

        x_cp.wait()
        x = jnp.broadcast_to(xbuf[0].astype(F32), (8, D))
        x = attention(x, True)
        x = mlp(x, True)
        if REP == 1:
            x = attention(x, False)
            x = mlp(x, False)
        else:
            def rep(i, x):
                x = attention(x, False)
                return mlp(x, False)
            x = lax.fori_loop(0, REP, rep, x)
        obuf[0] = x[0:1].astype(BF)
        o_cp.start()
        o_cp.wait()

    def fn(A_x, A_k_cache, A_v_cache, A_wq, A_wo, B_x, B_w1, B_w2, B_w3, B_w4):
        kT = _raw2(jnp.swapaxes(A_k_cache[0], 1, 2))
        vT = _raw2(jnp.swapaxes(A_v_cache[0], 1, 2))
        S = pltpu.VMEM((16, W // 2), F32)
        M = pltpu.VMEM((8, 128), F32)
        return pl.pallas_call(
            kernel,
            out_shape=jax.ShapeDtypeStruct((1, 1, D), BF),
            in_specs=[pl.BlockSpec(memory_space=pl.ANY)] * 7,
            out_specs=pl.BlockSpec(memory_space=pl.ANY),
            scratch_shapes=[
                pltpu.VMEM((H, 24, NCP, 8, 128), U32),
                pltpu.VMEM((H, 24, NCP, 8, 128), U32),
                pltpu.VMEM((80, 24, 8, 128), U32),
                pltpu.VMEM((384, 5, 8, 128), U32),
                pltpu.VMEM((D // 2, F), U32),
                pltpu.VMEM((F // 2, D), U32),
                pltpu.VMEM((128, 512), BF),
                S, S, S, S, M, M,
                pltpu.VMEM((PD, 128), F32),
                pltpu.VMEM((16, 128), F32),
                pltpu.VMEM((2, 2, 16, PD), BF),
                pltpu.VMEM((8, D), F32),
                pltpu.VMEM((8, PD), F32),
                pltpu.VMEM((8, D), BF),
                pltpu.VMEM((1, 1, D), BF),
                pltpu.VMEM((1, 1, D), BF),
                pltpu.SemaphoreType.DMA((H,)),
                pltpu.SemaphoreType.DMA((H,)),
                pltpu.SemaphoreType.DMA((5 + W4C,)),
            ],
            compiler_params=pltpu.CompilerParams(vmem_limit_bytes=127 * 2**20, flags=FLAGS),
        )(A_x, kT, vT, _raw2(A_wq), _raw5(A_wo), B_w3, B_w4)
    return fn


@jax.jit
def pallas_interleave_layers__sliding_block_cached__mixer_s_mlp__decode_kernel(
    A_x: jax.Array,
    A_k_cache: jax.Array,
    A_v_cache: jax.Array,
    A_wq: jax.Array,
    A_wo: jax.Array,
    B_x: jax.Array,
    B_w1: jax.Array,
    B_w2: jax.Array,
    B_w3: jax.Array,
    B_w4: jax.Array,
):
    sk = A_k_cache.shape[2]
    w = min(4096, max(256, sk // 4))
    return build(sk, w)(A_x, A_k_cache, A_v_cache, A_wq, A_wo, B_x, B_w1, B_w2, B_w3, B_w4)
```

```python
import jax
import jax.numpy as jnp
from jax import lax
import jax.experimental.pallas as pl
import jax.experimental.pallas.tpu as pltpu

D = 640
H = 32
DH = 192
F = 1536
NP = H // 2
PD = 2 * DH
LOG2E = 1.4426950408889634
EPS = 1e-5
BF = jnp.bfloat16
F32 = jnp.float32
U32 = jnp.uint32


def _ln(x):
    m = jnp.mean(x, axis=-1, keepdims=True)
    c = x - m
    v = jnp.mean(c * c, axis=-1, keepdims=True)
    return c * lax.rsqrt(v + EPS)


def _bf(w):
    return pltpu.bitcast(w, BF)


def _u(x):
    return pltpu.bitcast(x, U32)


def _raw2(a):
    *lead, r, c = a.shape
    n = len(lead)
    z = a.reshape(*lead, r // 8, 8, c // 256, 2, 128)
    z = z.transpose(*range(n), n, n + 2, n + 3, n + 1, n + 4)
    return z.reshape(*lead, r // 8, c // 256, 16, 128)


def _raw5(a):
    r, c = a.shape
    z = a.reshape(r // 8, 8, 5, 128).transpose(0, 2, 1, 3)
    return z.reshape(r // 16, 5, 16, 128)


FLAGS = None
def build(SK, W, NOCHK=1, DEPTH=2, REP=1, NA=2, MC=3, QA=10, QB=21, QAE=0, QBE=10, MA=16, MB=22, MK=0, EG=9, EGS=3, EGE=4, EGSE=2, FG=9, XK=2, W4C=4, LGRP=6, GR=23, ESK=2, PRIO=0):
    NCP = W // 256
    CP0 = (SK - W) // 256
    QSCALE = (DH ** -0.5) * LOG2E
    groups = [NA] * (24 // NA)
    NG = len(groups)
    NV = NCP - MC

    def kernel(x_hbm, k_hbm, v_hbm, wq_hbm, wo_hbm, w3_hbm, w4_hbm, o_hbm,
               kb, vb, wqb, wob, w3b, w4b, eca, sa, sb, ea, eb, mxa, mxb, accb, lb, Lb, xab, omb, xlb,
               xbuf, obuf, ksem, vsem, wsem):
        k32 = k_hbm.bitcast(U32)
        v32 = v_hbm.bitcast(U32)

        def kcp(p):
            return pltpu.make_async_copy(k32.at[pl.ds(2 * p, 2), :, pl.ds(CP0, NCP)], kb.at[pl.ds(2 * p, 2)], ksem.at[p])

        def vcp(p):
            return pltpu.make_async_copy(v32.at[pl.ds(2 * p, 2), :, pl.ds(CP0, NCP)], vb.at[pl.ds(2 * p, 2)], vsem.at[p])

        wq_cp = pltpu.make_async_copy(wq_hbm.bitcast(U32), wqb, wsem.at[0])
        wo_cp = pltpu.make_async_copy(wo_hbm.bitcast(U32), wob, wsem.at[1])
        w3_cp = pltpu.make_async_copy(w3_hbm.bitcast(U32), w3b, wsem.at[2])
        x_cp = pltpu.make_async_copy(x_hbm, xbuf, wsem.at[3])
        o_cp = pltpu.make_async_copy(obuf, o_hbm, wsem.at[4])
        R4 = F // 2 // W4C
        w4_cp = [pltpu.make_async_copy(w4_hbm.bitcast(U32).at[pl.ds(i * R4, R4)], w4b.at[pl.ds(i * R4, R4)], wsem.at[5 + i])
                 for i in range(W4C)]

        def issue_static(i):
            if i + 1 < NP:
                kcp(i + 1).start()
            vcp(i).start(priority=PRIO)
            if i == NP - 1:
                w3_cp.start()
                for c in w4_cp:
                    c.start()

        wq_cp.start()
        x_cp.start()
        kcp(0).start()
        wo_cp.start()
        for i in range(DEPTH):
            issue_static(i)

        low = lax.broadcasted_iota(jnp.int32, (8, 128), 0) < 4
        in_a = lax.broadcasted_iota(jnp.int32, (8, PD), 1) < DH

        def make_expand_matrix():
            row = lax.broadcasted_iota(jnp.int32, (128, 512), 0)
            col = lax.broadcasted_iota(jnp.int32, (128, 512), 1)
            hi = row >> 6
            jj = row & 63
            u = col >> 7
            cond = ((u >> 1) == hi) & ((col & 127) == ((jj >> 3) << 4) + ((u & 1) << 3) + (jj & 7))
            eca[...] = jnp.where(cond, 1.0, 0.0).astype(BF)

        def retile_wq():
            def body(g, _):
                for c in range(24):
                    a = wqb[2 * g, c]
                    b = wqb[2 * g + 1, c]
                    wqb[2 * g, c] = jnp.where(low, a, pltpu.roll(b, 4, 0))
                    wqb[2 * g + 1, c] = jnp.where(low, pltpu.roll(a, 4, 0), b)
                return _
            lax.fori_loop(0, 40, body, 0)

        def retile_wo():
            def body(gg, _):
                for u in range(4):
                    g = gg * 4 + u
                    raw = [wob[g, p] for p in range(5)]
                    rot = [pltpu.roll(r, 4, 0) for r in raw]
                    for c in range(5):
                        t1, t2 = c, 5 + c
                        top = raw[t1 // 2] if t1 % 2 == 0 else rot[t1 // 2]
                        bot = rot[t2 // 2] if t2 % 2 == 0 else raw[t2 // 2]
                        wob[g, c] = jnp.where(low, top, bot)
                return _
            lax.fori_loop(0, 96, body, 0)

        def qproj(p):
            cols = []
            for u in range(3):
                t = 3 * p + u
                w = wqb[pl.ds(t % 2, 40, stride=2), t // 2]
                cols.append(_bf(w.reshape(320, 128)))
            return jnp.dot(xlb[...], jnp.concatenate(cols, axis=1), preferred_element_type=F32)

        def expand(q):
            q = (q * QSCALE).astype(BF)
            qs = jnp.concatenate([q[:, 0:128], q[:, 128:256], q[:, 256:384]], axis=0)
            ex = jnp.dot(qs, eca[...], preferred_element_type=F32)

            def tile(t, hi):
                return jnp.concatenate([ex[t * 8:(t + 1) * 8, (2 * hi) * 128:(2 * hi + 1) * 128],
                                        ex[t * 8:(t + 1) * 8, (2 * hi + 1) * 128:(2 * hi + 2) * 128]], axis=0)
            la = jnp.concatenate([tile(0, 0), tile(0, 1), tile(1, 0)], axis=1).astype(BF)
            lb_ = jnp.concatenate([tile(1, 1), tile(2, 0), tile(2, 1)], axis=1).astype(BF)
            return la, lb_

        def transpose_v(p):
            def body(ci, _):
                c = NV + ci
                nat = [[], []]
                for hh in range(2):
                    raw = [vb[2 * p + hh, r, c] for r in range(24)]
                    for g in range(12):
                        a, b = raw[2 * g], raw[2 * g + 1]
                        nat[0].append(jnp.where(low, a, pltpu.roll(b, 4, 0)))
                        nat[1].append(jnp.where(low, pltpu.roll(a, 4, 0), b))
                outs = []
                for cc in range(2):
                    t = _u(_bf(jnp.concatenate(nat[cc], axis=0)).T)
                    for j in range(3):
                        for mm in range(8):
                            outs.append(t[mm * 8:(mm + 1) * 8, j * 128:(j + 1) * 128])
                for s_, v in enumerate(outs):
                    vb[2 * p + s_ // 24, s_ % 24, c] = v
                return _
            lax.fori_loop(0, MC, body, 0)

        def pv_mxu(p, ea_, eb_, gates, z):
            lhs = []
            rhs = []
            for ci in range(MC):
                c = NV + ci
                for cc in range(2):
                    k = 2 * ci + cc
                    lhs.append(jnp.concatenate([ea_[cc * 8:(cc + 1) * 8, c * 128:(c + 1) * 128],
                                                eb_[cc * 8:(cc + 1) * 8, c * 128:(c + 1) * 128]], axis=0))
                    fz = _u(gates[min(MA + ((MB - MA) * k) // (2 * MC), len(gates) - 1)]) & z
                    cols = []
                    for j in range(3):
                        rows = []
                        for mm in range(8):
                            s_ = (cc * 3 + j) * 8 + mm
                            v = vb[2 * p + s_ // 24, s_ % 24, c]
                            rows.append(v | fz if (mm == 7 and j == 0) else v)
                        cols.append(jnp.concatenate(rows, axis=0))
                    rhs.append(jnp.concatenate(cols, axis=1))
            e = jnp.concatenate(lhs, axis=1).astype(BF)
            out = jnp.dot(e, _bf(jnp.concatenate(rhs, axis=0)), preferred_element_type=F32)
            return jnp.where(in_a, out[0:8], out[8:16])

        def qk(h, L, dst, mxd, gates=None, z=None, cb=None, qa=0, qb=0, xk=None):
            ms = []
            for c in range(NCP):
                w = kb[h, :, c]
                if gates is not None:
                    gi = min(qa + ((qb - qa) * c) // NCP, len(gates) - 1)
                    fz = _u(gates[gi]) & z
                    w = jnp.concatenate([w[r] | fz if r == GR else w[r] for r in range(24)], axis=0)
                else:
                    w = w.reshape(192, 128)
                s = jnp.dot(L, _bf(w), preferred_element_type=F32)
                dst[:, c * 128:(c + 1) * 128] = s
                ms.append(s)
                if cb is not None and c == (XK if xk is None else xk):
                    cb()
            m = ms[0]
            for t in ms[1:]:
                m = jnp.maximum(m, t)
            mxd[...] = jnp.maximum(m[0:8], m[8:16])

        def expo(src, mxs, edst):
            mh = jnp.broadcast_to(jnp.max(mxs[...], axis=1, keepdims=True), (8, 128))
            parts = []
            for c in range(NCP):
                e0 = jnp.exp2(src[0:8, c * 128:(c + 1) * 128] - mh)
                e1 = jnp.exp2(src[8:16, c * 128:(c + 1) * 128] - mh)
                edst[0:8, c * 128:(c + 1) * 128] = e0
                edst[8:16, c * 128:(c + 1) * 128] = e1
                parts.append(e1)
            return parts

        def pv(h, esrc, par, eparts, pre, z, prev):
            eg, egs = (EGE, EGSE) if par == 0 else (EG, EGS)
            r0 = 0
            outs = []
            l = jnp.zeros((8, 128), F32)
            for gi, na in enumerate(groups):
                deps = []
                if prev is not None:
                    deps.append(prev[0])
                if eg <= gi < eg + egs:
                    k0 = ((gi - eg) * NCP) // egs
                    k1 = ((gi - eg + 1) * NCP) // egs
                    for k in range(k0, k1):
                        if (k - k0) % ESK == ESK - 1 or k == k1 - 1:
                            deps.append(eparts[k])
                for pg, val in pre:
                    if pg == gi:
                        deps.append(val)
                if deps:
                    t = _u(deps[0])
                    for dd in deps[1:]:
                        t = t | _u(dd)
                    acc0 = pltpu.bitcast(t & z, F32)
                else:
                    acc0 = jnp.zeros((8, 128), F32)
                acc = [acc0 for _ in range(na)]
                for c in range(NCP):
                    if c >= NV and gi != LGRP:
                        continue
                    e0 = esrc[0:8, c * 128:(c + 1) * 128]
                    e1 = esrc[8:16, c * 128:(c + 1) * 128]
                    if gi == LGRP:
                        l = l + (e0 + e1)
                    if c >= NV:
                        continue
                    for r in range(na):
                        f = _bf(vb[h, r0 + r, c]).astype(F32)
                        acc[r] = acc[r] + (f[0:8] * e0 + f[8:16] * e1)
                for r in range(na):
                    accb[par * 192 + (r0 + r) * 8: par * 192 + (r0 + r) * 8 + 8, :] = acc[r]
                r0 += na
                prev = acc
                outs.append(acc[0])
            lb[par * 8:(par + 1) * 8, :] = l
            return outs

        def finish():
            o = jnp.sum(accb[...].T, axis=0, keepdims=True)
            inv = 1.0 / jnp.sum(lb[...], axis=1, keepdims=True)
            o = (o + omb[...]) * jnp.where(in_a, inv[0:8], inv[8:16])
            return o

        def wo_dot(o, p):
            g0 = pl.multiple_of(p * 24, 8)
            cols = [_bf(wob[pl.ds(g0, 24), c].reshape(192, 128)) for c in range(5)]
            return jnp.dot(o.astype(BF), jnp.concatenate(cols, axis=1), preferred_element_type=F32)

        def block(p):
            z = jnp.broadcast_to(lax.shift_right_arithmetic(p, 31), (8, 128)).astype(U32)
            p1 = jnp.minimum(p + 1, NP - 1)
            p2 = jnp.minimum(p + 2, NP - 1)
            le = Lb[p1 % 2, 0]
            lo = Lb[p1 % 2, 1]
            q = qproj(p2)

            def cb():
                la, lb_ = expand(q)
                Lb[p2 % 2, 0] = la
                Lb[p2 % 2, 1] = lb_
            o = finish()
            pre = [(FG, o[:, 0:128])] if FG else []
            ge = pv(2 * p, ea, 0, expo(sa, mxa, eb), pre, z, None)
            qk(2 * p1, le, sb, mxb, ge, z, cb, QAE, QBE)
            xab[...] += wo_dot(o, jnp.maximum(p - 1, 0))
            if MK == 0:
                ea_v = {(c, cc): None for c in range(NV, NCP) for cc in range(2)}
            ea_keep = ea[:, NV * 128:NCP * 128]
            go = pv(2 * p + 1, eb, 1, expo(sb, mxb, ea), [], z, [ge[-1]])
            gates = ge + go

            class _Shift:
                def __getitem__(self, idx):
                    r, c = idx
                    return ea_keep[r, c.start - NV * 128:c.stop - NV * 128]
            if MK == 0:
                qk(2 * p1 + 1, lo, sa, mxa, gates, z, None, QA, QB)
                omb[...] = pv_mxu(p, _Shift(), eb, gates, z)
            else:
                def cb2():
                    omb[...] = pv_mxu(p, _Shift(), eb, gates, z)
                qk(2 * p1 + 1, lo, sa, mxa, gates, z, cb2, QA, QB, MK)

        def attention(x, first):
            xlb[...] = _ln(x).astype(BF)
            if first:
                make_expand_matrix()
                wq_cp.wait()
                retile_wq()
            q0 = qproj(0)
            q1 = qproj(1)
            la, lb_ = expand(q0)
            la1, lb1 = expand(q1)
            Lb[1, 0] = la1
            Lb[1, 1] = lb1
            if first:
                kcp(0).wait()
            qk(0, la, sb, mxb)
            qk(1, lb_, sa, mxa)
            expo(sb, mxb, ea)
            xab[...] = jnp.zeros_like(xab)
            accb[...] = jnp.zeros_like(accb)
            lb[...] = jnp.ones_like(lb)
            omb[...] = jnp.zeros_like(omb)
            if first:
                wo_cp.wait()
                retile_wo()

            def body(p, carry):
                if first:
                    @pl.when(p + 1 < NP)
                    def _():
                        kcp(p + 1).wait()
                    vcp(p).wait()

                    @pl.when(p + DEPTH < NP)
                    def _():
                        i = p + DEPTH

                        @pl.when(i + 1 < NP)
                        def _():
                            kcp(i + 1).start()
                        vcp(i).start(priority=PRIO)

                        @pl.when(i == NP - 1)
                        def _():
                            w3_cp.start()
                            for c in w4_cp:
                                c.start()

                    transpose_v(p)
                block(p)
                return carry

            lax.fori_loop(0, NP, body, 0)
            return x + xab[...] + wo_dot(finish(), NP - 1)

        def mlp(x, first):
            u = _ln(x)
            h = _ln(u).astype(BF)
            if first:
                w3_cp.wait()
            g = jnp.dot(h, _bf(w3b[...]), preferred_element_type=F32)
            g = jax.nn.gelu(g, approximate=True).astype(BF)
            y = x + u
            if first:
                for i in range(W4C):
                    w4_cp[i].wait()
                    y = y + jnp.dot(g[:, i * 2 * R4:(i + 1) * 2 * R4], _bf(w4b[i * R4:(i + 1) * R4, :]), preferred_element_type=F32)
            else:
                y = y + jnp.dot(g, _bf(w4b[...]), preferred_element_type=F32)
            return y

        x_cp.wait()
        x = jnp.broadcast_to(xbuf[0].astype(F32), (8, D))
        x = attention(x, True)
        x = mlp(x, True)
        if REP == 1:
            x = attention(x, False)
            x = mlp(x, False)
        else:
            def rep(i, x):
                x = attention(x, False)
                return mlp(x, False)
            x = lax.fori_loop(0, REP, rep, x)
        obuf[0] = x[0:1].astype(BF)
        o_cp.start()
        o_cp.wait()

    def fn(A_x, A_k_cache, A_v_cache, A_wq, A_wo, B_x, B_w1, B_w2, B_w3, B_w4):
        kT = _raw2(jnp.swapaxes(A_k_cache[0], 1, 2))
        vT = _raw2(jnp.swapaxes(A_v_cache[0], 1, 2))
        S = pltpu.VMEM((16, W // 2), F32)
        M = pltpu.VMEM((8, 128), F32)
        return pl.pallas_call(
            kernel,
            out_shape=jax.ShapeDtypeStruct((1, 1, D), BF),
            in_specs=[pl.BlockSpec(memory_space=pl.ANY)] * 7,
            out_specs=pl.BlockSpec(memory_space=pl.ANY),
            scratch_shapes=[
                pltpu.VMEM((H, 24, NCP, 8, 128), U32),
                pltpu.VMEM((H, 24, NCP, 8, 128), U32),
                pltpu.VMEM((80, 24, 8, 128), U32),
                pltpu.VMEM((384, 5, 8, 128), U32),
                pltpu.VMEM((D // 2, F), U32),
                pltpu.VMEM((F // 2, D), U32),
                pltpu.VMEM((128, 512), BF),
                S, S, S, S, M, M,
                pltpu.VMEM((PD, 128), F32),
                pltpu.VMEM((16, 128), F32),
                pltpu.VMEM((2, 2, 16, PD), BF),
                pltpu.VMEM((8, D), F32),
                pltpu.VMEM((8, PD), F32),
                pltpu.VMEM((8, D), BF),
                pltpu.VMEM((1, 1, D), BF),
                pltpu.VMEM((1, 1, D), BF),
                pltpu.SemaphoreType.DMA((NP,)),
                pltpu.SemaphoreType.DMA((NP,)),
                pltpu.SemaphoreType.DMA((5 + W4C,)),
            ],
            compiler_params=pltpu.CompilerParams(vmem_limit_bytes=127 * 2**20, flags=FLAGS, disable_semaphore_checks=bool(NOCHK)),
        )(A_x, kT, vT, _raw2(A_wq), _raw5(A_wo), B_w3, B_w4)
    return fn


@jax.jit
def pallas_interleave_layers__sliding_block_cached__mixer_s_mlp__decode_kernel(
    A_x: jax.Array,
    A_k_cache: jax.Array,
    A_v_cache: jax.Array,
    A_wq: jax.Array,
    A_wo: jax.Array,
    B_x: jax.Array,
    B_w1: jax.Array,
    B_w2: jax.Array,
    B_w3: jax.Array,
    B_w4: jax.Array,
):
    sk = A_k_cache.shape[2]
    w = min(4096, max(256, sk // 4))
    return build(sk, w)(A_x, A_k_cache, A_v_cache, A_wq, A_wo, B_x, B_w1, B_w2, B_w3, B_w4)
```

```python
import jax
import jax.numpy as jnp
from jax import lax
import jax.experimental.pallas as pl
import jax.experimental.pallas.tpu as pltpu

D = 640
H = 32
DH = 192
F = 1536
NP = H // 2
PD = 2 * DH
LOG2E = 1.4426950408889634
EPS = 1e-5
BF = jnp.bfloat16
F32 = jnp.float32
U32 = jnp.uint32

DEPTH = 2
W4C = 4
MC = 3
NA = 2
NG = 24 // NA
QAE, QBE = -4, 9
QA, QB = 8, 21
MA, MB = 16, 22
EGE, EGSE = 5, 2
EG, EGS = 10, 2
FG = 8
XK = 10
LGRP = 6
GR = 15
ESK = 8


def _moments(x):
    m = jnp.mean(x, axis=-1, keepdims=True)
    v = jnp.maximum(jnp.mean(x * x, axis=-1, keepdims=True) - m * m, 0.0)
    return m, v


def _ln(x):
    m, v = _moments(x)
    return (x - m) * lax.rsqrt(v + EPS)


def _ln_ln(x):
    m, v = _moments(x)
    r = lax.rsqrt(v + EPS)
    u = (x - m) * r
    return u, u * lax.rsqrt(v * r * r + EPS)


def _bf(w):
    return pltpu.bitcast(w, BF)


def _u(x):
    return pltpu.bitcast(x, U32)


def _raw2(a):
    *lead, r, c = a.shape
    n = len(lead)
    z = a.reshape(*lead, r // 8, 8, c // 256, 2, 128)
    z = z.transpose(*range(n), n, n + 2, n + 3, n + 1, n + 4)
    return z.reshape(*lead, r // 8, c // 256, 16, 128)


def _raw5(a):
    r, c = a.shape
    z = a.reshape(r // 8, 8, 5, 128).transpose(0, 2, 1, 3)
    return z.reshape(r // 16, 5, 16, 128)


def build(SK, W, REP=1):
    assert W % 256 == 0 and (SK - W) % 256 == 0
    NCP = W // 256
    CP0 = (SK - W) // 256
    NV = NCP - MC
    QSCALE = (DH ** -0.5) * LOG2E
    R4 = F // 2 // W4C

    def kernel(x_hbm, k_hbm, v_hbm, wq_hbm, wo_hbm, w3_hbm, w4_hbm, o_hbm,
               kb, vb, wqb, wob, w3b, w4b, eca, sa, sb, ea, eb, mxa, mxb, accb, lb, Lb, xab, omb, xlb,
               xbuf, obuf, ksem, vsem, wsem):
        k32 = k_hbm.bitcast(U32)
        v32 = v_hbm.bitcast(U32)

        def kcp(p):
            return pltpu.make_async_copy(k32.at[pl.ds(2 * p, 2), :, pl.ds(CP0, NCP)], kb.at[pl.ds(2 * p, 2)], ksem.at[p])

        def vcp(p):
            return pltpu.make_async_copy(v32.at[pl.ds(2 * p, 2), :, pl.ds(CP0, NCP)], vb.at[pl.ds(2 * p, 2)], vsem.at[p])

        wq_cp = pltpu.make_async_copy(wq_hbm.bitcast(U32), wqb, wsem.at[0])
        wo_cp = pltpu.make_async_copy(wo_hbm.bitcast(U32), wob, wsem.at[1])
        w3_cp = pltpu.make_async_copy(w3_hbm.bitcast(U32), w3b, wsem.at[2])
        x_cp = pltpu.make_async_copy(x_hbm, xbuf, wsem.at[3])
        o_cp = pltpu.make_async_copy(obuf, o_hbm, wsem.at[4])
        w4_cp = [pltpu.make_async_copy(w4_hbm.bitcast(U32).at[pl.ds(i * R4, R4)], w4b.at[pl.ds(i * R4, R4)], wsem.at[5 + i])
                 for i in range(W4C)]

        wq_cp.start()
        x_cp.start()
        kcp(0).start()
        wo_cp.start()
        for i in range(DEPTH):
            kcp(i + 1).start()
            vcp(i).start()

        low = lax.broadcasted_iota(jnp.int32, (8, 128), 0) < 4
        in_a = lax.broadcasted_iota(jnp.int32, (8, PD), 1) < DH

        def make_expand_matrix():
            row = lax.broadcasted_iota(jnp.int32, (128, 512), 0)
            col = lax.broadcasted_iota(jnp.int32, (128, 512), 1)
            hi = row >> 6
            jj = row & 63
            u = col >> 7
            cond = ((u >> 1) == hi) & ((col & 127) == ((jj >> 3) << 4) + ((u & 1) << 3) + (jj & 7))
            eca[...] = jnp.where(cond, 1.0, 0.0).astype(BF)

        def retile_wq():
            def body(g, _):
                for c in range(24):
                    a = wqb[g, 0, c]
                    b = wqb[g, 1, c]
                    wqb[g, 0, c] = jnp.where(low, a, pltpu.roll(b, 4, 0))
                    wqb[g, 1, c] = jnp.where(low, pltpu.roll(a, 4, 0), b)
                return _
            lax.fori_loop(0, 40, body, 0)

        def retile_wo():
            def body(gg, _):
                for u in range(4):
                    g = gg * 4 + u
                    raw = [wob[g, p] for p in range(5)]
                    rot = [pltpu.roll(r, 4, 0) for r in raw]
                    for c in range(5):
                        t1, t2 = c, 5 + c
                        top = raw[t1 // 2] if t1 % 2 == 0 else rot[t1 // 2]
                        bot = rot[t2 // 2] if t2 % 2 == 0 else raw[t2 // 2]
                        wob[g, c] = jnp.where(low, top, bot)
                return _
            lax.fori_loop(0, 96, body, 0)

        def transpose_v(p):
            def body(ci, _):
                c = NV + ci
                nat = [[], []]
                for hh in range(2):
                    raw = [vb[2 * p + hh, r, c] for r in range(24)]
                    for g in range(12):
                        a, b = raw[2 * g], raw[2 * g + 1]
                        nat[0].append(jnp.where(low, a, pltpu.roll(b, 4, 0)))
                        nat[1].append(jnp.where(low, pltpu.roll(a, 4, 0), b))
                outs = []
                for cc in range(2):
                    t = _u(_bf(jnp.concatenate(nat[cc], axis=0)).T)
                    for j in range(3):
                        for mm in range(8):
                            outs.append(t[mm * 8:(mm + 1) * 8, j * 128:(j + 1) * 128])
                for s, v in enumerate(outs):
                    vb[2 * p + s // 24, s % 24, c] = v
                return _
            lax.fori_loop(0, MC, body, 0)

        def qproj(p):
            cols = []
            for u in range(3):
                t = 3 * p + u
                cols.append(_bf(wqb[:, t % 2, t // 2].reshape(320, 128)))
            return jnp.dot(xlb[...], jnp.concatenate(cols, axis=1), preferred_element_type=F32)

        def expand(q):
            q = (q * QSCALE).astype(BF)
            qs = jnp.concatenate([q[:, 0:128], q[:, 128:256], q[:, 256:384]], axis=0)
            ex = jnp.dot(qs, eca[...], preferred_element_type=F32)

            def tile(t, hi):
                return jnp.concatenate([ex[t * 8:(t + 1) * 8, (2 * hi) * 128:(2 * hi + 1) * 128],
                                        ex[t * 8:(t + 1) * 8, (2 * hi + 1) * 128:(2 * hi + 2) * 128]], axis=0)
            la = jnp.concatenate([tile(0, 0), tile(0, 1), tile(1, 0)], axis=1).astype(BF)
            lb_ = jnp.concatenate([tile(1, 1), tile(2, 0), tile(2, 1)], axis=1).astype(BF)
            return la, lb_

        def qk(h, L, dst, mxd, gates=None, z=None, qa=0, qb=0, cb=None):
            ms = []
            for c in range(NCP):
                w = kb[h, :, c]
                gi = -1 if gates is None else min(qa + ((qb - qa) * c) // NCP, len(gates) - 1)
                if gi >= 0:
                    fz = _u(gates[gi]) & z
                    w = jnp.concatenate([w[r] | fz if r == GR else w[r] for r in range(24)], axis=0)
                else:
                    w = w.reshape(192, 128)
                s = jnp.dot(L, _bf(w), preferred_element_type=F32)
                dst[:, c * 128:(c + 1) * 128] = s
                ms.append(s)
                if cb is not None and c == XK:
                    cb()
            m = ms[0]
            for t in ms[1:]:
                m = jnp.maximum(m, t)
            mxd[...] = jnp.maximum(m[0:8], m[8:16])

        def expo(src, mxs, edst):
            mh = jnp.broadcast_to(jnp.max(mxs[...], axis=1, keepdims=True), (8, 128))
            parts = []
            for c in range(NCP):
                e0 = jnp.exp2(src[0:8, c * 128:(c + 1) * 128] - mh)
                e1 = jnp.exp2(src[8:16, c * 128:(c + 1) * 128] - mh)
                edst[0:8, c * 128:(c + 1) * 128] = e0
                edst[8:16, c * 128:(c + 1) * 128] = e1
                parts.append(e1)
            return parts

        def pv_vpu(h, esrc, par, eparts, pre, z, prev):
            eg, egs = (EGE, EGSE) if par == 0 else (EG, EGS)
            outs = []
            l = jnp.zeros((8, 128), F32)
            for gi in range(NG):
                deps = []
                if prev is not None:
                    deps.append(prev[0])
                if eg <= gi < eg + egs:
                    k0 = ((gi - eg) * NCP) // egs
                    k1 = ((gi - eg + 1) * NCP) // egs
                    for k in range(k0, k1):
                        if (k - k0) % ESK == ESK - 1 or k == k1 - 1:
                            deps.append(eparts[k])
                for pg, val in pre:
                    if pg == gi:
                        deps.append(val)
                if deps:
                    t = _u(deps[0])
                    for dd in deps[1:]:
                        t = t | _u(dd)
                    acc0 = pltpu.bitcast(t & z, F32)
                else:
                    acc0 = jnp.zeros((8, 128), F32)
                acc = [acc0 for _ in range(NA)]
                for c in range(NCP):
                    if c >= NV and gi != LGRP:
                        continue
                    e0 = esrc[0:8, c * 128:(c + 1) * 128]
                    e1 = esrc[8:16, c * 128:(c + 1) * 128]
                    if gi == LGRP:
                        l = l + (e0 + e1)
                    if c >= NV:
                        continue
                    for r in range(NA):
                        f = _bf(vb[h, gi * NA + r, c]).astype(F32)
                        acc[r] = acc[r] + (f[0:8] * e0 + f[8:16] * e1)
                for r in range(NA):
                    r0 = par * DH + (gi * NA + r) * 8
                    accb[r0:r0 + 8, :] = acc[r]
                prev = acc
                outs.append(acc[0])
            lb[par * 8:(par + 1) * 8, :] = l
            return outs

        def pv_mxu(p, e_even, e_odd, gates, z):
            lhs = []
            rhs = []
            for ci in range(MC):
                c = NV + ci
                for cc in range(2):
                    lhs.append(jnp.concatenate([e_even[cc * 8:(cc + 1) * 8, ci * 128:(ci + 1) * 128],
                                                e_odd[cc * 8:(cc + 1) * 8, c * 128:(c + 1) * 128]], axis=0))
                    fz = _u(gates[min(MA + ((MB - MA) * (2 * ci + cc)) // (2 * MC), len(gates) - 1)]) & z
                    cols = []
                    for j in range(3):
                        rows = []
                        for mm in range(8):
                            s = (cc * 3 + j) * 8 + mm
                            v = vb[2 * p + s // 24, s % 24, c]
                            rows.append(v | fz if (mm == 7 and j == 0) else v)
                        cols.append(jnp.concatenate(rows, axis=0))
                    rhs.append(jnp.concatenate(cols, axis=1))
            e = jnp.concatenate(lhs, axis=1).astype(BF)
            out = jnp.dot(e, _bf(jnp.concatenate(rhs, axis=0)), preferred_element_type=F32)
            return jnp.where(in_a, out[0:8], out[8:16])

        def finish():
            o = jnp.sum(accb[...].T, axis=0, keepdims=True)
            inv = 1.0 / jnp.sum(lb[...], axis=1, keepdims=True)
            return (o + omb[...]) * jnp.where(in_a, inv[0:8], inv[8:16])

        def wo_dot(o, p):
            g0 = pl.multiple_of(p * 24, 8)
            cols = [_bf(wob[pl.ds(g0, 24), c].reshape(192, 128)) for c in range(5)]
            return jnp.dot(o.astype(BF), jnp.concatenate(cols, axis=1), preferred_element_type=F32)

        def block(p):
            z = jnp.broadcast_to(lax.shift_right_arithmetic(p, 31), (8, 128)).astype(U32)
            p1 = jnp.minimum(p + 1, NP - 1)
            p2 = jnp.minimum(p + 2, NP - 1)
            le = Lb[p1 % 2, 0]
            lo = Lb[p1 % 2, 1]
            q = qproj(p2)

            def issue_expand():
                la, lb_ = expand(q)
                Lb[p2 % 2, 0] = la
                Lb[p2 % 2, 1] = lb_
            o = finish()
            ge = pv_vpu(2 * p, ea, 0, expo(sa, mxa, eb), [(FG, o[:, 0:128])], z, None)
            qk(2 * p1, le, sb, mxb, ge, z, QAE, QBE, issue_expand)
            xab[...] += wo_dot(o, jnp.maximum(p - 1, 0))
            e_even = ea[:, NV * 128:NCP * 128]
            go = pv_vpu(2 * p + 1, eb, 1, expo(sb, mxb, ea), [], z, [ge[-1]])
            qk(2 * p1 + 1, lo, sa, mxa, ge + go, z, QA, QB)
            omb[...] = pv_mxu(p, e_even, eb, ge + go, z)

        def attention(x, first):
            xlb[...] = _ln(x).astype(BF)
            if first:
                make_expand_matrix()
                wq_cp.wait()
                retile_wq()
            q0 = qproj(0)
            q1 = qproj(1)
            la, lb_ = expand(q0)
            la1, lb1 = expand(q1)
            Lb[1, 0] = la1
            Lb[1, 1] = lb1
            if first:
                kcp(0).wait()
            qk(0, la, sb, mxb)
            qk(1, lb_, sa, mxa)
            expo(sb, mxb, ea)
            xab[...] = jnp.zeros_like(xab)
            accb[...] = jnp.zeros_like(accb)
            lb[...] = jnp.ones_like(lb)
            omb[...] = jnp.zeros_like(omb)
            if first:
                wo_cp.wait()
                retile_wo()

            def body(p, carry):
                if first:
                    @pl.when(p + 1 < NP)
                    def _():
                        kcp(p + 1).wait()
                    vcp(p).wait()

                    @pl.when(p + DEPTH < NP)
                    def _():
                        i = p + DEPTH

                        @pl.when(i + 1 < NP)
                        def _():
                            kcp(i + 1).start()
                        vcp(i).start()

                        @pl.when(i == NP - 1)
                        def _():
                            w3_cp.start()
                            for c in w4_cp:
                                c.start()

                    transpose_v(p)
                block(p)
                return carry

            lax.fori_loop(0, NP, body, 0)
            return x + xab[...] + wo_dot(finish(), NP - 1)

        def mlp(x, first):
            u, h = _ln_ln(x)
            if first:
                w3_cp.wait()
            g = jnp.dot(h.astype(BF), _bf(w3b[...]), preferred_element_type=F32)
            g = jax.nn.gelu(g, approximate=True).astype(BF)
            y = x + u
            if first:
                for i in range(W4C):
                    w4_cp[i].wait()
                    y = y + jnp.dot(g[:, i * 2 * R4:(i + 1) * 2 * R4], _bf(w4b[i * R4:(i + 1) * R4, :]),
                                    preferred_element_type=F32)
            else:
                y = y + jnp.dot(g, _bf(w4b[...]), preferred_element_type=F32)
            return y

        x_cp.wait()
        x = jnp.broadcast_to(xbuf[0].astype(F32), (8, D))
        x = attention(x, True)
        x = mlp(x, True)
        if REP == 1:
            x = attention(x, False)
            x = mlp(x, False)
        else:
            x = lax.fori_loop(0, REP, lambda i, x: mlp(attention(x, False), False), x)
        obuf[0] = x[0:1].astype(BF)
        o_cp.start()
        o_cp.wait()

    def fn(A_x, A_k_cache, A_v_cache, A_wq, A_wo, B_x, B_w1, B_w2, B_w3, B_w4):
        kT = _raw2(jnp.swapaxes(A_k_cache[0], 1, 2))
        vT = _raw2(jnp.swapaxes(A_v_cache[0], 1, 2))
        S = pltpu.VMEM((16, W // 2), F32)
        M = pltpu.VMEM((8, 128), F32)
        return pl.pallas_call(
            kernel,
            out_shape=jax.ShapeDtypeStruct((1, 1, D), BF),
            in_specs=[pl.BlockSpec(memory_space=pl.ANY)] * 7,
            out_specs=pl.BlockSpec(memory_space=pl.ANY),
            scratch_shapes=[
                pltpu.VMEM((H, 24, NCP, 8, 128), U32),
                pltpu.VMEM((H, 24, NCP, 8, 128), U32),
                pltpu.VMEM((40, 2, 24, 8, 128), U32),
                pltpu.VMEM((384, 5, 8, 128), U32),
                pltpu.VMEM((D // 2, F), U32),
                pltpu.VMEM((F // 2, D), U32),
                pltpu.VMEM((128, 512), BF),
                S, S, S, S, M, M,
                pltpu.VMEM((PD, 128), F32),
                pltpu.VMEM((16, 128), F32),
                pltpu.VMEM((2, 2, 16, PD), BF),
                pltpu.VMEM((8, D), F32),
                pltpu.VMEM((8, PD), F32),
                pltpu.VMEM((8, D), BF),
                pltpu.VMEM((1, 1, D), BF),
                pltpu.VMEM((1, 1, D), BF),
                pltpu.SemaphoreType.DMA((NP,)),
                pltpu.SemaphoreType.DMA((NP,)),
                pltpu.SemaphoreType.DMA((5 + W4C,)),
            ],
            compiler_params=pltpu.CompilerParams(vmem_limit_bytes=127 * 2**20, disable_semaphore_checks=True),
        )(A_x, kT, vT, _raw2(A_wq).reshape(40, 2, 24, 16, 128), _raw5(A_wo), B_w3, B_w4)
    return fn


@jax.jit
def pallas_interleave_layers__sliding_block_cached__mixer_s_mlp__decode_kernel(
    A_x: jax.Array,
    A_k_cache: jax.Array,
    A_v_cache: jax.Array,
    A_wq: jax.Array,
    A_wo: jax.Array,
    B_x: jax.Array,
    B_w1: jax.Array,
    B_w2: jax.Array,
    B_w3: jax.Array,
    B_w4: jax.Array,
):
    sk = A_k_cache.shape[2]
    w = min(4096, max(256, sk // 4))
    return build(sk, w)(A_x, A_k_cache, A_v_cache, A_wq, A_wo, B_x, B_w1, B_w2, B_w3, B_w4)
```

```python
import jax
import jax.numpy as jnp
from jax import lax
import jax.experimental.pallas as pl
import jax.experimental.pallas.tpu as pltpu

D = 640
H = 32
DH = 192
F = 1536
NP = H // 2
PD = 2 * DH
LOG2E = 1.4426950408889634
EPS = 1e-5
BF = jnp.bfloat16
F32 = jnp.float32
U32 = jnp.uint32

DEPTH = 2
W4C = 4
MC = 3
NA = 2
NG = 24 // NA
QAE, QBE = -4, 9
QA, QB = 11, 21
MA, MB = 18, 23
EGE, EGSE = 5, 1
EG, EGS = 9, 2
FG = 8
XK = 10
LGRP = 10
GR = 7
ESK = 16
PPK = 1
CD = 1
CD0 = 4


def _moments(x):
    m = jnp.mean(x, axis=-1, keepdims=True)
    v = jnp.maximum(jnp.mean(x * x, axis=-1, keepdims=True) - m * m, 0.0)
    return m, v


def _ln(x):
    m, v = _moments(x)
    return (x - m) * lax.rsqrt(v + EPS)


def _ln_ln(x):
    m, v = _moments(x)
    r = lax.rsqrt(v + EPS)
    u = (x - m) * r
    return u, u * lax.rsqrt(v * r * r + EPS)


def _bf(w):
    return pltpu.bitcast(w, BF)


def _u(x):
    return pltpu.bitcast(x, U32)


def _raw2(a):
    *lead, r, c = a.shape
    n = len(lead)
    z = a.reshape(*lead, r // 8, 8, c // 256, 2, 128)
    z = z.transpose(*range(n), n, n + 2, n + 3, n + 1, n + 4)
    return z.reshape(*lead, r // 8, c // 256, 16, 128)


def _raw5(a):
    r, c = a.shape
    z = a.reshape(r // 8, 8, 5, 128).transpose(0, 2, 1, 3)
    return z.reshape(r // 16, 5, 16, 128)


def build(SK, W, REP=1):
    assert W % 256 == 0 and (SK - W) % 256 == 0
    NCP = W // 256
    CP0 = (SK - W) // 256
    NV = NCP - MC
    QSCALE = (DH ** -0.5) * LOG2E
    R4 = F // 2 // W4C

    def kernel(x_hbm, k_hbm, v_hbm, wq_hbm, wo_hbm, w3_hbm, w4_hbm, o_hbm,
               kb, vb, vf, wqb, wob, w3b, w4b, eca, sa, sb, ea, eb, mxa, mxb, accb, lb, Lb, xab, omb, xlb,
               xbuf, obuf, ksem, vsem, wsem):
        k32 = k_hbm.bitcast(U32)
        v32 = v_hbm.bitcast(U32)

        def kcp(p):
            return pltpu.make_async_copy(k32.at[pl.ds(2 * p, 2), :, pl.ds(CP0, NCP)], kb.at[pl.ds(2 * p, 2)], ksem.at[p])

        def vcp(p):
            return pltpu.make_async_copy(v32.at[pl.ds(2 * p, 2), :, pl.ds(CP0, NCP)], vb.at[pl.ds(2 * p, 2)], vsem.at[p])

        wq_cp = pltpu.make_async_copy(wq_hbm.bitcast(U32), wqb, wsem.at[0])
        wo_cp = pltpu.make_async_copy(wo_hbm.bitcast(U32), wob, wsem.at[1])
        w3_cp = pltpu.make_async_copy(w3_hbm.bitcast(U32), w3b, wsem.at[2])
        x_cp = pltpu.make_async_copy(x_hbm, xbuf, wsem.at[3])
        o_cp = pltpu.make_async_copy(obuf, o_hbm, wsem.at[4])
        w4_cp = [pltpu.make_async_copy(w4_hbm.bitcast(U32).at[pl.ds(i * R4, R4)], w4b.at[pl.ds(i * R4, R4)], wsem.at[5 + i])
                 for i in range(W4C)]

        wq_cp.start()
        x_cp.start()
        kcp(0).start()
        wo_cp.start()
        for i in range(DEPTH):
            kcp(i + 1).start()
            vcp(i).start()

        low = lax.broadcasted_iota(jnp.int32, (8, 128), 0) < 4
        in_a = lax.broadcasted_iota(jnp.int32, (8, PD), 1) < DH

        def make_expand_matrix():
            row = lax.broadcasted_iota(jnp.int32, (128, 512), 0)
            col = lax.broadcasted_iota(jnp.int32, (128, 512), 1)
            hi = row >> 6
            jj = row & 63
            u = col >> 7
            cond = ((u >> 1) == hi) & ((col & 127) == ((jj >> 3) << 4) + ((u & 1) << 3) + (jj & 7))
            eca[...] = jnp.where(cond, 1.0, 0.0).astype(BF)

        def retile_wq():
            def body(g, _):
                for c in range(24):
                    a = wqb[g, 0, c]
                    b = wqb[g, 1, c]
                    wqb[g, 0, c] = jnp.where(low, a, pltpu.roll(b, 4, 0))
                    wqb[g, 1, c] = jnp.where(low, pltpu.roll(a, 4, 0), b)
                return _
            lax.fori_loop(0, 40, body, 0)

        def retile_wo():
            def body(gg, _):
                for u in range(4):
                    g = gg * 4 + u
                    raw = [wob[g, p] for p in range(5)]
                    rot = [pltpu.roll(r, 4, 0) for r in raw]
                    for c in range(5):
                        t1, t2 = c, 5 + c
                        top = raw[t1 // 2] if t1 % 2 == 0 else rot[t1 // 2]
                        bot = rot[t2 // 2] if t2 % 2 == 0 else raw[t2 // 2]
                        wob[g, c] = jnp.where(low, top, bot)
                return _
            lax.fori_loop(0, 96, body, 0)

        def transpose_v(p):
            def body(ci, _):
                c = NV + ci
                nat = [[], []]
                for hh in range(2):
                    raw = [vb[2 * p + hh, r, c] for r in range(24)]
                    for g in range(12):
                        a, b = raw[2 * g], raw[2 * g + 1]
                        nat[0].append(jnp.where(low, a, pltpu.roll(b, 4, 0)))
                        nat[1].append(jnp.where(low, pltpu.roll(a, 4, 0), b))
                outs = []
                for cc in range(2):
                    t = _u(_bf(jnp.concatenate(nat[cc], axis=0)).T)
                    for j in range(3):
                        for mm in range(8):
                            outs.append(t[mm * 8:(mm + 1) * 8, j * 128:(j + 1) * 128])
                for s, v in enumerate(outs):
                    vb[2 * p + s // 24, s % 24, c] = v
                return _
            lax.fori_loop(0, MC, body, 0)

        def widen_v(p):
            def body(hh, _):
                h = 2 * p + hh
                for c in range(PPK):
                    for r in range(24):
                        f = _bf(vb[h, r, c]).astype(F32)
                        vf[h, r, c, 0] = f[0:8]
                        vf[h, r, c, 1] = f[8:16]
                return _
            lax.fori_loop(0, 2, body, 0)

        def qproj(p):
            cols = []
            for u in range(3):
                t = 3 * p + u
                cols.append(_bf(wqb[:, t % 2, t // 2].reshape(320, 128)))
            return jnp.dot(xlb[...], jnp.concatenate(cols, axis=1), preferred_element_type=F32)

        def expand(q):
            q = (q * QSCALE).astype(BF)
            qs = jnp.concatenate([q[:, 0:128], q[:, 128:256], q[:, 256:384]], axis=0)
            ex = jnp.dot(qs, eca[...], preferred_element_type=F32)

            def tile(t, hi):
                return jnp.concatenate([ex[t * 8:(t + 1) * 8, (2 * hi) * 128:(2 * hi + 1) * 128],
                                        ex[t * 8:(t + 1) * 8, (2 * hi + 1) * 128:(2 * hi + 2) * 128]], axis=0)
            la = jnp.concatenate([tile(0, 0), tile(0, 1), tile(1, 0)], axis=1).astype(BF)
            lb_ = jnp.concatenate([tile(1, 1), tile(2, 0), tile(2, 1)], axis=1).astype(BF)
            return la, lb_

        def qk(h, L, dst, mxd, gates=None, z=None, qa=0, qb=0, cb=None):
            ms = []
            for c in range(NCP):
                w = kb[h, :, c]
                gi = -1 if gates is None else min(qa + ((qb - qa) * c) // NCP, len(gates) - 1)
                if gi >= 0:
                    fz = _u(gates[gi]) & z
                    w = jnp.concatenate([w[r] | fz if r == GR else w[r] for r in range(24)], axis=0)
                else:
                    w = w.reshape(192, 128)
                s = jnp.dot(L, _bf(w), preferred_element_type=F32)
                dst[:, c * 128:(c + 1) * 128] = s
                ms.append(s)
                if cb is not None and c == XK:
                    cb()
            m = ms[0]
            for t in ms[1:]:
                m = jnp.maximum(m, t)
            mxd[...] = jnp.maximum(m[0:8], m[8:16])

        def expo(src, mxs, edst):
            mh = jnp.broadcast_to(jnp.max(mxs[...], axis=1, keepdims=True), (8, 128))
            parts = []
            for c in range(NCP):
                e0 = jnp.exp2(src[0:8, c * 128:(c + 1) * 128] - mh)
                e1 = jnp.exp2(src[8:16, c * 128:(c + 1) * 128] - mh)
                edst[0:8, c * 128:(c + 1) * 128] = e0
                edst[8:16, c * 128:(c + 1) * 128] = e1
                parts.append(e1)
            return parts

        def pv_vpu(h, esrc, par, eparts, pre, z, prev):
            hist = list(prev) if prev is not None else []
            eg, egs = (EGE, EGSE) if par == 0 else (EG, EGS)
            outs = []
            l = jnp.zeros((8, 128), F32)
            for gi in range(NG):
                deps = []
                if len(hist) >= CD and not (par == 0 and gi < CD0):
                    deps.append(hist[-CD])
                if eg <= gi < eg + egs:
                    k0 = ((gi - eg) * NCP) // egs
                    k1 = ((gi - eg + 1) * NCP) // egs
                    for k in range(k0, k1):
                        if (k - k0) % ESK == ESK - 1 or k == k1 - 1:
                            deps.append(eparts[k])
                for pg, val in pre:
                    if pg == gi:
                        deps.append(val)
                if deps:
                    t = _u(deps[0])
                    for dd in deps[1:]:
                        t = t | _u(dd)
                    acc0 = pltpu.bitcast(t & z, F32)
                else:
                    acc0 = jnp.zeros((8, 128), F32)
                acc = [acc0 for _ in range(NA)]
                for c in range(NCP):
                    if c >= NV and gi != LGRP:
                        continue
                    e0 = esrc[0:8, c * 128:(c + 1) * 128]
                    e1 = esrc[8:16, c * 128:(c + 1) * 128]
                    if gi == LGRP:
                        l = l + (e0 + e1)
                    if c >= NV:
                        continue
                    for r in range(NA):
                        if c < PPK:
                            f0, f1 = vf[h, gi * NA + r, c, 0], vf[h, gi * NA + r, c, 1]
                        else:
                            f = _bf(vb[h, gi * NA + r, c]).astype(F32)
                            f0, f1 = f[0:8], f[8:16]
                        acc[r] = acc[r] + (f0 * e0 + f1 * e1)
                for r in range(NA):
                    r0 = par * DH + (gi * NA + r) * 8
                    accb[r0:r0 + 8, :] = acc[r]
                hist.append(acc[0])
                outs.append(acc[0])
            lb[par * 8:(par + 1) * 8, :] = l
            return outs

        def pv_mxu(p, e_even, e_odd, gates, z):
            lhs = []
            rhs = []
            for ci in range(MC):
                c = NV + ci
                for cc in range(2):
                    lhs.append(jnp.concatenate([e_even[cc * 8:(cc + 1) * 8, ci * 128:(ci + 1) * 128],
                                                e_odd[cc * 8:(cc + 1) * 8, c * 128:(c + 1) * 128]], axis=0))
                    fz = _u(gates[min(MA + ((MB - MA) * (2 * ci + cc)) // (2 * MC), len(gates) - 1)]) & z
                    cols = []
                    for j in range(3):
                        rows = []
                        for mm in range(8):
                            s = (cc * 3 + j) * 8 + mm
                            v = vb[2 * p + s // 24, s % 24, c]
                            rows.append(v | fz if (mm == 7 and j == 0) else v)
                        cols.append(jnp.concatenate(rows, axis=0))
                    rhs.append(jnp.concatenate(cols, axis=1))
            e = jnp.concatenate(lhs, axis=1).astype(BF)
            out = jnp.dot(e, _bf(jnp.concatenate(rhs, axis=0)), preferred_element_type=F32)
            return jnp.where(in_a, out[0:8], out[8:16])

        def finish():
            o = jnp.sum(accb[...].T, axis=0, keepdims=True)
            inv = 1.0 / jnp.sum(lb[...], axis=1, keepdims=True)
            return (o + omb[...]) * jnp.where(in_a, inv[0:8], inv[8:16])

        def wo_dot(o, p):
            g0 = pl.multiple_of(p * 24, 8)
            cols = [_bf(wob[pl.ds(g0, 24), c].reshape(192, 128)) for c in range(5)]
            return jnp.dot(o.astype(BF), jnp.concatenate(cols, axis=1), preferred_element_type=F32)

        def block(p):
            z = jnp.broadcast_to(lax.shift_right_arithmetic(p, 31), (8, 128)).astype(U32)
            p1 = jnp.minimum(p + 1, NP - 1)
            p2 = jnp.minimum(p + 2, NP - 1)
            le = Lb[p1 % 2, 0]
            lo = Lb[p1 % 2, 1]
            q = qproj(p2)

            def issue_expand():
                la, lb_ = expand(q)
                Lb[p2 % 2, 0] = la
                Lb[p2 % 2, 1] = lb_
            o = finish()
            ge = pv_vpu(2 * p, ea, 0, expo(sa, mxa, eb), [(FG, o[:, 0:128])], z, None)
            qk(2 * p1, le, sb, mxb, ge, z, QAE, QBE, issue_expand)
            xab[...] += wo_dot(o, jnp.maximum(p - 1, 0))
            e_even = ea[:, NV * 128:NCP * 128]
            go = pv_vpu(2 * p + 1, eb, 1, expo(sb, mxb, ea), [], z, ge)
            qk(2 * p1 + 1, lo, sa, mxa, ge + go, z, QA, QB)
            omb[...] = pv_mxu(p, e_even, eb, ge + go, z)

        def attention(x, first):
            xlb[...] = _ln(x).astype(BF)
            if first:
                make_expand_matrix()
                wq_cp.wait()
                retile_wq()
            q0 = qproj(0)
            q1 = qproj(1)
            la, lb_ = expand(q0)
            la1, lb1 = expand(q1)
            Lb[1, 0] = la1
            Lb[1, 1] = lb1
            if first:
                kcp(0).wait()
            qk(0, la, sb, mxb)
            qk(1, lb_, sa, mxa)
            expo(sb, mxb, ea)
            xab[...] = jnp.zeros_like(xab)
            accb[...] = jnp.zeros_like(accb)
            lb[...] = jnp.ones_like(lb)
            omb[...] = jnp.zeros_like(omb)
            if first:
                wo_cp.wait()
                retile_wo()

            def body(p, carry):
                if first:
                    @pl.when(p + 1 < NP)
                    def _():
                        kcp(p + 1).wait()
                    vcp(p).wait()

                    @pl.when(p + DEPTH < NP)
                    def _():
                        i = p + DEPTH

                        @pl.when(i + 1 < NP)
                        def _():
                            kcp(i + 1).start()
                        vcp(i).start()

                        @pl.when(i == NP - 1)
                        def _():
                            w3_cp.start()
                            for c in w4_cp:
                                c.start()

                    transpose_v(p)
                    if PPK:
                        widen_v(p)
                block(p)
                return carry

            lax.fori_loop(0, NP, body, 0)
            return x + xab[...] + wo_dot(finish(), NP - 1)

        def mlp(x, first):
            u, h = _ln_ln(x)
            if first:
                w3_cp.wait()
            g = jnp.dot(h.astype(BF), _bf(w3b[...]), preferred_element_type=F32)
            g = jax.nn.gelu(g, approximate=True).astype(BF)
            y = x + u
            if first:
                for i in range(W4C):
                    w4_cp[i].wait()
                    y = y + jnp.dot(g[:, i * 2 * R4:(i + 1) * 2 * R4], _bf(w4b[i * R4:(i + 1) * R4, :]),
                                    preferred_element_type=F32)
            else:
                y = y + jnp.dot(g, _bf(w4b[...]), preferred_element_type=F32)
            return y

        x_cp.wait()
        x = jnp.broadcast_to(xbuf[0].astype(F32), (8, D))
        x = attention(x, True)
        x = mlp(x, True)
        if REP == 1:
            x = attention(x, False)
            x = mlp(x, False)
        else:
            x = lax.fori_loop(0, REP, lambda i, x: mlp(attention(x, False), False), x)
        obuf[0] = x[0:1].astype(BF)
        o_cp.start()
        o_cp.wait()

    def fn(A_x, A_k_cache, A_v_cache, A_wq, A_wo, B_x, B_w1, B_w2, B_w3, B_w4):
        kT = _raw2(jnp.swapaxes(A_k_cache[0], 1, 2))
        vT = _raw2(jnp.swapaxes(A_v_cache[0], 1, 2))
        S = pltpu.VMEM((16, W // 2), F32)
        M = pltpu.VMEM((8, 128), F32)
        return pl.pallas_call(
            kernel,
            out_shape=jax.ShapeDtypeStruct((1, 1, D), BF),
            in_specs=[pl.BlockSpec(memory_space=pl.ANY)] * 7,
            out_specs=pl.BlockSpec(memory_space=pl.ANY),
            scratch_shapes=[
                pltpu.VMEM((H, 24, NCP, 8, 128), U32),
                pltpu.VMEM((H, 24, NCP, 8, 128), U32),
                pltpu.VMEM((H, 24, max(PPK, 1), 2, 8, 128), F32),
                pltpu.VMEM((40, 2, 24, 8, 128), U32),
                pltpu.VMEM((384, 5, 8, 128), U32),
                pltpu.VMEM((D // 2, F), U32),
                pltpu.VMEM((F // 2, D), U32),
                pltpu.VMEM((128, 512), BF),
                S, S, S, S, M, M,
                pltpu.VMEM((PD, 128), F32),
                pltpu.VMEM((16, 128), F32),
                pltpu.VMEM((2, 2, 16, PD), BF),
                pltpu.VMEM((8, D), F32),
                pltpu.VMEM((8, PD), F32),
                pltpu.VMEM((8, D), BF),
                pltpu.VMEM((1, 1, D), BF),
                pltpu.VMEM((1, 1, D), BF),
                pltpu.SemaphoreType.DMA((NP,)),
                pltpu.SemaphoreType.DMA((NP,)),
                pltpu.SemaphoreType.DMA((5 + W4C,)),
            ],
            compiler_params=pltpu.CompilerParams(vmem_limit_bytes=127 * 2**20, disable_semaphore_checks=True),
        )(A_x, kT, vT, _raw2(A_wq).reshape(40, 2, 24, 16, 128), _raw5(A_wo), B_w3, B_w4)
    return fn


@jax.jit
def pallas_interleave_layers__sliding_block_cached__mixer_s_mlp__decode_kernel(
    A_x: jax.Array,
    A_k_cache: jax.Array,
    A_v_cache: jax.Array,
    A_wq: jax.Array,
    A_wo: jax.Array,
    B_x: jax.Array,
    B_w1: jax.Array,
    B_w2: jax.Array,
    B_w3: jax.Array,
    B_w4: jax.Array,
):
    sk = A_k_cache.shape[2]
    w = min(4096, max(256, sk // 4))
    return build(sk, w)(A_x, A_k_cache, A_v_cache, A_wq, A_wo, B_x, B_w1, B_w2, B_w3, B_w4)
```

```python
import jax
import jax.numpy as jnp
from jax import lax
import jax.experimental.pallas as pl
import jax.experimental.pallas.tpu as pltpu

D = 640
H = 32
DH = 192
F = 1536
NP = H // 2
PD = 2 * DH
LOG2E = 1.4426950408889634
EPS = 1e-5
BF = jnp.bfloat16
F32 = jnp.float32
U32 = jnp.uint32

DEPTH = 2
W4C = 4
MC = 3
NA = 2
NG = 24 // NA
QAE, QBE = -4, 9
QA, QB = 11, 21
MA, MB = 18, 23
EGE, EGSE = 5, 1
EG, EGS = 9, 2
FG = 8
XK = 10
LGRP = 10
GR = 7
ESK = 16
PPK = 1
CD = 1
CD0 = 4


def _moments(x):
    m = jnp.mean(x, axis=-1, keepdims=True)
    v = jnp.maximum(jnp.mean(x * x, axis=-1, keepdims=True) - m * m, 0.0)
    return m, v


def _ln(x):
    m, v = _moments(x)
    return (x - m) * lax.rsqrt(v + EPS)


def _ln_ln(x):
    m, v = _moments(x)
    r = lax.rsqrt(v + EPS)
    u = (x - m) * r
    return u, u * lax.rsqrt(v * r * r + EPS)


def _bf(w):
    return pltpu.bitcast(w, BF)


def _u(x):
    return pltpu.bitcast(x, U32)


def _raw2(a):
    *lead, r, c = a.shape
    n = len(lead)
    z = a.reshape(*lead, r // 8, 8, c // 256, 2, 128)
    z = z.transpose(*range(n), n, n + 2, n + 3, n + 1, n + 4)
    return z.reshape(*lead, r // 8, c // 256, 16, 128)


def _raw5(a):
    r, c = a.shape
    z = a.reshape(r // 8, 8, 5, 128).transpose(0, 2, 1, 3)
    return z.reshape(r // 16, 5, 16, 128)


def build(SK, W):
    assert W % 256 == 0 and (SK - W) % 256 == 0
    NCP = W // 256
    CP0 = (SK - W) // 256
    NV = NCP - MC
    QSCALE = (DH ** -0.5) * LOG2E
    R4 = F // 2 // W4C

    def kernel(x_hbm, k_hbm, v_hbm, wq_hbm, wo_hbm, w3_hbm, w4_hbm, o_hbm,
               kb, vb, vf, wqb, wob, w3b, w4b, eca, sa, sb, ea, eb, mxa, mxb, accb, lb, Lb, xab, omb, xlb,
               xbuf, obuf, ksem, vsem, wsem):
        k32 = k_hbm.bitcast(U32)
        v32 = v_hbm.bitcast(U32)

        def kcp(p):
            return pltpu.make_async_copy(k32.at[pl.ds(2 * p, 2), :, pl.ds(CP0, NCP)], kb.at[pl.ds(2 * p, 2)], ksem.at[p])

        def vcp(p):
            return pltpu.make_async_copy(v32.at[pl.ds(2 * p, 2), :, pl.ds(CP0, NCP)], vb.at[pl.ds(2 * p, 2)], vsem.at[p])

        wq_cp = pltpu.make_async_copy(wq_hbm.bitcast(U32), wqb, wsem.at[0])
        wo_cp = pltpu.make_async_copy(wo_hbm.bitcast(U32), wob, wsem.at[1])
        w3_cp = pltpu.make_async_copy(w3_hbm.bitcast(U32), w3b, wsem.at[2])
        x_cp = pltpu.make_async_copy(x_hbm, xbuf, wsem.at[3])
        o_cp = pltpu.make_async_copy(obuf, o_hbm, wsem.at[4])
        w4_cp = [pltpu.make_async_copy(w4_hbm.bitcast(U32).at[pl.ds(i * R4, R4)], w4b.at[pl.ds(i * R4, R4)], wsem.at[5 + i])
                 for i in range(W4C)]

        wq_cp.start()
        x_cp.start()
        kcp(0).start()
        wo_cp.start()
        for i in range(DEPTH):
            kcp(i + 1).start()
            vcp(i).start()

        low = lax.broadcasted_iota(jnp.int32, (8, 128), 0) < 4
        in_a = lax.broadcasted_iota(jnp.int32, (8, PD), 1) < DH

        def make_expand_matrix():
            row = lax.broadcasted_iota(jnp.int32, (128, 512), 0)
            col = lax.broadcasted_iota(jnp.int32, (128, 512), 1)
            hi = row >> 6
            jj = row & 63
            u = col >> 7
            cond = ((u >> 1) == hi) & ((col & 127) == ((jj >> 3) << 4) + ((u & 1) << 3) + (jj & 7))
            eca[...] = jnp.where(cond, 1.0, 0.0).astype(BF)

        def retile_wq():
            def body(g, _):
                for c in range(24):
                    a = wqb[g, 0, c]
                    b = wqb[g, 1, c]
                    wqb[g, 0, c] = jnp.where(low, a, pltpu.roll(b, 4, 0))
                    wqb[g, 1, c] = jnp.where(low, pltpu.roll(a, 4, 0), b)
                return _
            lax.fori_loop(0, 40, body, 0)

        def retile_wo():
            def body(gg, _):
                for u in range(4):
                    g = gg * 4 + u
                    raw = [wob[g, p] for p in range(5)]
                    rot = [pltpu.roll(r, 4, 0) for r in raw]
                    for c in range(5):
                        t1, t2 = c, 5 + c
                        top = raw[t1 // 2] if t1 % 2 == 0 else rot[t1 // 2]
                        bot = rot[t2 // 2] if t2 % 2 == 0 else raw[t2 // 2]
                        wob[g, c] = jnp.where(low, top, bot)
                return _
            lax.fori_loop(0, 96, body, 0)

        def transpose_v(p):
            def body(ci, _):
                c = NV + ci
                nat = [[], []]
                for hh in range(2):
                    raw = [vb[2 * p + hh, r, c] for r in range(24)]
                    for g in range(12):
                        a, b = raw[2 * g], raw[2 * g + 1]
                        nat[0].append(jnp.where(low, a, pltpu.roll(b, 4, 0)))
                        nat[1].append(jnp.where(low, pltpu.roll(a, 4, 0), b))
                outs = []
                for cc in range(2):
                    t = _u(_bf(jnp.concatenate(nat[cc], axis=0)).T)
                    for j in range(3):
                        for mm in range(8):
                            outs.append(t[mm * 8:(mm + 1) * 8, j * 128:(j + 1) * 128])
                for s, v in enumerate(outs):
                    vb[2 * p + s // 24, s % 24, c] = v
                return _
            lax.fori_loop(0, MC, body, 0)

        def widen_v(p):
            def body(hh, _):
                h = 2 * p + hh
                for c in range(PPK):
                    for r in range(24):
                        f = _bf(vb[h, r, c]).astype(F32)
                        vf[h, r, c, 0] = f[0:8]
                        vf[h, r, c, 1] = f[8:16]
                return _
            lax.fori_loop(0, 2, body, 0)

        def qproj(p):
            cols = []
            for u in range(3):
                t = 3 * p + u
                cols.append(_bf(wqb[:, t % 2, t // 2].reshape(320, 128)))
            return jnp.dot(xlb[...], jnp.concatenate(cols, axis=1), preferred_element_type=F32)

        def expand(q):
            q = (q * QSCALE).astype(BF)
            qs = jnp.concatenate([q[:, 0:128], q[:, 128:256], q[:, 256:384]], axis=0)
            ex = jnp.dot(qs, eca[...], preferred_element_type=F32)

            def tile(t, hi):
                return jnp.concatenate([ex[t * 8:(t + 1) * 8, (2 * hi) * 128:(2 * hi + 1) * 128],
                                        ex[t * 8:(t + 1) * 8, (2 * hi + 1) * 128:(2 * hi + 2) * 128]], axis=0)
            la = jnp.concatenate([tile(0, 0), tile(0, 1), tile(1, 0)], axis=1).astype(BF)
            lb_ = jnp.concatenate([tile(1, 1), tile(2, 0), tile(2, 1)], axis=1).astype(BF)
            return la, lb_

        def qk(h, L, dst, mxd, gates=None, z=None, qa=0, qb=0, cb=None):
            ms = []
            for c in range(NCP):
                w = kb[h, :, c]
                gi = -1 if gates is None else min(qa + ((qb - qa) * c) // NCP, len(gates) - 1)
                if gi >= 0:
                    fz = _u(gates[gi]) & z
                    w = jnp.concatenate([w[r] | fz if r == GR else w[r] for r in range(24)], axis=0)
                else:
                    w = w.reshape(192, 128)
                s = jnp.dot(L, _bf(w), preferred_element_type=F32)
                dst[:, c * 128:(c + 1) * 128] = s
                ms.append(s)
                if cb is not None and c == XK:
                    cb()
            m = ms[0]
            for t in ms[1:]:
                m = jnp.maximum(m, t)
            mxd[...] = jnp.maximum(m[0:8], m[8:16])

        def expo(src, mxs, edst):
            mh = jnp.broadcast_to(jnp.max(mxs[...], axis=1, keepdims=True), (8, 128))
            parts = []
            for c in range(NCP):
                e0 = jnp.exp2(src[0:8, c * 128:(c + 1) * 128] - mh)
                e1 = jnp.exp2(src[8:16, c * 128:(c + 1) * 128] - mh)
                edst[0:8, c * 128:(c + 1) * 128] = e0
                edst[8:16, c * 128:(c + 1) * 128] = e1
                parts.append(e1)
            return parts

        def pv_vpu(h, esrc, par, eparts, pre, z, prev):
            hist = list(prev) if prev is not None else []
            eg, egs = (EGE, EGSE) if par == 0 else (EG, EGS)
            outs = []
            l = jnp.zeros((8, 128), F32)
            for gi in range(NG):
                deps = []
                if len(hist) >= CD and not (par == 0 and gi < CD0):
                    deps.append(hist[-CD])
                if eg <= gi < eg + egs:
                    k0 = ((gi - eg) * NCP) // egs
                    k1 = ((gi - eg + 1) * NCP) // egs
                    for k in range(k0, k1):
                        if (k - k0) % ESK == ESK - 1 or k == k1 - 1:
                            deps.append(eparts[k])
                for pg, val in pre:
                    if pg == gi:
                        deps.append(val)
                if deps:
                    t = _u(deps[0])
                    for dd in deps[1:]:
                        t = t | _u(dd)
                    acc0 = pltpu.bitcast(t & z, F32)
                else:
                    acc0 = jnp.zeros((8, 128), F32)
                acc = [acc0 for _ in range(NA)]
                for c in range(NCP):
                    if c >= NV and gi != LGRP:
                        continue
                    e0 = esrc[0:8, c * 128:(c + 1) * 128]
                    e1 = esrc[8:16, c * 128:(c + 1) * 128]
                    if gi == LGRP:
                        l = l + (e0 + e1)
                    if c >= NV:
                        continue
                    for r in range(NA):
                        if c < PPK:
                            f0, f1 = vf[h, gi * NA + r, c, 0], vf[h, gi * NA + r, c, 1]
                        else:
                            f = _bf(vb[h, gi * NA + r, c]).astype(F32)
                            f0, f1 = f[0:8], f[8:16]
                        acc[r] = acc[r] + (f0 * e0 + f1 * e1)
                for r in range(NA):
                    r0 = par * DH + (gi * NA + r) * 8
                    accb[r0:r0 + 8, :] = acc[r]
                hist.append(acc[0])
                outs.append(acc[0])
            lb[par * 8:(par + 1) * 8, :] = l
            return outs

        def pv_mxu(p, e_even, e_odd, gates, z):
            lhs = []
            rhs = []
            for ci in range(MC):
                c = NV + ci
                for cc in range(2):
                    lhs.append(jnp.concatenate([e_even[cc * 8:(cc + 1) * 8, ci * 128:(ci + 1) * 128],
                                                e_odd[cc * 8:(cc + 1) * 8, c * 128:(c + 1) * 128]], axis=0))
                    fz = _u(gates[min(MA + ((MB - MA) * (2 * ci + cc)) // (2 * MC), len(gates) - 1)]) & z
                    cols = []
                    for j in range(3):
                        rows = []
                        for mm in range(8):
                            s = (cc * 3 + j) * 8 + mm
                            v = vb[2 * p + s // 24, s % 24, c]
                            rows.append(v | fz if (mm == 7 and j == 0) else v)
                        cols.append(jnp.concatenate(rows, axis=0))
                    rhs.append(jnp.concatenate(cols, axis=1))
            e = jnp.concatenate(lhs, axis=1).astype(BF)
            out = jnp.dot(e, _bf(jnp.concatenate(rhs, axis=0)), preferred_element_type=F32)
            return jnp.where(in_a, out[0:8], out[8:16])

        def finish():
            o = jnp.sum(accb[...].T, axis=0, keepdims=True)
            inv = 1.0 / jnp.sum(lb[...], axis=1, keepdims=True)
            return (o + omb[...]) * jnp.where(in_a, inv[0:8], inv[8:16])

        def wo_dot(o, p):
            g0 = pl.multiple_of(p * 24, 8)
            cols = [_bf(wob[pl.ds(g0, 24), c].reshape(192, 128)) for c in range(5)]
            return jnp.dot(o.astype(BF), jnp.concatenate(cols, axis=1), preferred_element_type=F32)

        def block(p):
            z = jnp.broadcast_to(lax.shift_right_arithmetic(p, 31), (8, 128)).astype(U32)
            p1 = jnp.minimum(p + 1, NP - 1)
            p2 = jnp.minimum(p + 2, NP - 1)
            le = Lb[p1 % 2, 0]
            lo = Lb[p1 % 2, 1]
            q = qproj(p2)

            def issue_expand():
                la, lb_ = expand(q)
                Lb[p2 % 2, 0] = la
                Lb[p2 % 2, 1] = lb_
            o = finish()
            ge = pv_vpu(2 * p, ea, 0, expo(sa, mxa, eb), [(FG, o[:, 0:128])], z, None)
            qk(2 * p1, le, sb, mxb, ge, z, QAE, QBE, issue_expand)
            xab[...] += wo_dot(o, jnp.maximum(p - 1, 0))
            e_even = ea[:, NV * 128:NCP * 128]
            go = pv_vpu(2 * p + 1, eb, 1, expo(sb, mxb, ea), [], z, ge)
            qk(2 * p1 + 1, lo, sa, mxa, ge + go, z, QA, QB)
            omb[...] = pv_mxu(p, e_even, eb, ge + go, z)

        def attention(x, first):
            xlb[...] = _ln(x).astype(BF)
            if first:
                make_expand_matrix()
                wq_cp.wait()
                retile_wq()
            q0 = qproj(0)
            q1 = qproj(1)
            la, lb_ = expand(q0)
            la1, lb1 = expand(q1)
            Lb[1, 0] = la1
            Lb[1, 1] = lb1
            if first:
                kcp(0).wait()
            qk(0, la, sb, mxb)
            qk(1, lb_, sa, mxa)
            expo(sb, mxb, ea)
            xab[...] = jnp.zeros_like(xab)
            accb[...] = jnp.zeros_like(accb)
            lb[...] = jnp.ones_like(lb)
            omb[...] = jnp.zeros_like(omb)
            if first:
                wo_cp.wait()
                retile_wo()

            def body(p, carry):
                if first:
                    @pl.when(p + 1 < NP)
                    def _():
                        kcp(p + 1).wait()
                    vcp(p).wait()

                    @pl.when(p + DEPTH < NP)
                    def _():
                        i = p + DEPTH

                        @pl.when(i + 1 < NP)
                        def _():
                            kcp(i + 1).start()
                        vcp(i).start()

                        @pl.when(i == NP - 1)
                        def _():
                            w3_cp.start()
                            for c in w4_cp:
                                c.start()

                    transpose_v(p)
                    if PPK:
                        widen_v(p)
                block(p)
                return carry

            lax.fori_loop(0, NP, body, 0)
            return x + xab[...] + wo_dot(finish(), NP - 1)

        def mlp(x, first):
            u, h = _ln_ln(x)
            if first:
                w3_cp.wait()
            g = jnp.dot(h.astype(BF), _bf(w3b[...]), preferred_element_type=F32)
            g = jax.nn.gelu(g, approximate=True).astype(BF)
            y = x + u
            if first:
                for i in range(W4C):
                    w4_cp[i].wait()
                    y = y + jnp.dot(g[:, i * 2 * R4:(i + 1) * 2 * R4], _bf(w4b[i * R4:(i + 1) * R4, :]),
                                    preferred_element_type=F32)
            else:
                y = y + jnp.dot(g, _bf(w4b[...]), preferred_element_type=F32)
            return y

        x_cp.wait()
        x = jnp.broadcast_to(xbuf[0].astype(F32), (8, D))
        x = attention(x, True)
        x = mlp(x, True)
        x = attention(x, False)
        x = mlp(x, False)
        obuf[0] = x[0:1].astype(BF)
        o_cp.start()
        o_cp.wait()

    def fn(A_x, A_k_cache, A_v_cache, A_wq, A_wo, B_x, B_w1, B_w2, B_w3, B_w4):
        kT = _raw2(jnp.swapaxes(A_k_cache[0], 1, 2))
        vT = _raw2(jnp.swapaxes(A_v_cache[0], 1, 2))
        S = pltpu.VMEM((16, W // 2), F32)
        M = pltpu.VMEM((8, 128), F32)
        return pl.pallas_call(
            kernel,
            out_shape=jax.ShapeDtypeStruct((1, 1, D), BF),
            in_specs=[pl.BlockSpec(memory_space=pl.ANY)] * 7,
            out_specs=pl.BlockSpec(memory_space=pl.ANY),
            scratch_shapes=[
                pltpu.VMEM((H, 24, NCP, 8, 128), U32),
                pltpu.VMEM((H, 24, NCP, 8, 128), U32),
                pltpu.VMEM((H, 24, max(PPK, 1), 2, 8, 128), F32),
                pltpu.VMEM((40, 2, 24, 8, 128), U32),
                pltpu.VMEM((384, 5, 8, 128), U32),
                pltpu.VMEM((D // 2, F), U32),
                pltpu.VMEM((F // 2, D), U32),
                pltpu.VMEM((128, 512), BF),
                S, S, S, S, M, M,
                pltpu.VMEM((PD, 128), F32),
                pltpu.VMEM((16, 128), F32),
                pltpu.VMEM((2, 2, 16, PD), BF),
                pltpu.VMEM((8, D), F32),
                pltpu.VMEM((8, PD), F32),
                pltpu.VMEM((8, D), BF),
                pltpu.VMEM((1, 1, D), BF),
                pltpu.VMEM((1, 1, D), BF),
                pltpu.SemaphoreType.DMA((NP,)),
                pltpu.SemaphoreType.DMA((NP,)),
                pltpu.SemaphoreType.DMA((5 + W4C,)),
            ],
            compiler_params=pltpu.CompilerParams(vmem_limit_bytes=127 * 2**20, disable_semaphore_checks=True),
        )(A_x, kT, vT, _raw2(A_wq).reshape(40, 2, 24, 16, 128), _raw5(A_wo), B_w3, B_w4)
    return fn


@jax.jit
def pallas_interleave_layers__sliding_block_cached__mixer_s_mlp__decode_kernel(
    A_x: jax.Array,
    A_k_cache: jax.Array,
    A_v_cache: jax.Array,
    A_wq: jax.Array,
    A_wo: jax.Array,
    B_x: jax.Array,
    B_w1: jax.Array,
    B_w2: jax.Array,
    B_w3: jax.Array,
    B_w4: jax.Array,
):
    sk = A_k_cache.shape[2]
    w = min(4096, max(256, sk // 4))
    return build(sk, w)(A_x, A_k_cache, A_v_cache, A_wq, A_wo, B_x, B_w1, B_w2, B_w3, B_w4)
```

```python
import jax
import jax.numpy as jnp
from jax import lax
import jax.experimental.pallas as pl
import jax.experimental.pallas.tpu as pltpu

D = 640
H = 32
DH = 192
F = 1536
NP = H // 2
PD = 2 * DH
LOG2E = 1.4426950408889634
EPS = 1e-5
BF = jnp.bfloat16
F32 = jnp.float32
U32 = jnp.uint32

DEPTH = 2
W4C = 4
MC = 3
NA = 2
NG = 24 // NA
QAE, QBE = -6, 9
QA, QB = 11, 20
MA, MB = 16, 22
EGE, EGSE = 5, 1
EG, EGS = 10, 2
FG = 8
XK = 10
LGRP = 9
GR = 15
ESK = 16
PPK = 1
CD = 1
CD0 = 5


def _moments(x):
    m = jnp.mean(x, axis=-1, keepdims=True)
    v = jnp.maximum(jnp.mean(x * x, axis=-1, keepdims=True) - m * m, 0.0)
    return m, v


def _ln(x):
    m, v = _moments(x)
    return (x - m) * lax.rsqrt(v + EPS)


def _ln_ln(x):
    m, v = _moments(x)
    r = lax.rsqrt(v + EPS)
    u = (x - m) * r
    return u, u * lax.rsqrt(v * r * r + EPS)


def _bf(w):
    return pltpu.bitcast(w, BF)


def _u(x):
    return pltpu.bitcast(x, U32)


def _raw2(a):
    *lead, r, c = a.shape
    n = len(lead)
    z = a.reshape(*lead, r // 8, 8, c // 256, 2, 128)
    z = z.transpose(*range(n), n, n + 2, n + 3, n + 1, n + 4)
    return z.reshape(*lead, r // 8, c // 256, 16, 128)


def _raw5(a):
    r, c = a.shape
    z = a.reshape(r // 8, 8, 5, 128).transpose(0, 2, 1, 3)
    return z.reshape(r // 16, 5, 16, 128)


def build(SK, W):
    assert W % 256 == 0 and (SK - W) % 256 == 0
    NCP = W // 256
    CP0 = (SK - W) // 256
    NV = NCP - MC
    QSCALE = (DH ** -0.5) * LOG2E
    R4 = F // 2 // W4C

    def kernel(x_hbm, k_hbm, v_hbm, wq_hbm, wo_hbm, w3_hbm, w4_hbm, o_hbm,
               kb, vb, vf, wqb, wob, w3b, w4b, eca, sa, sb, ea, eb, mxa, mxb, accb, lb, Lb, xab, omb, xlb,
               xbuf, obuf, ksem, vsem, wsem):
        k32 = k_hbm.bitcast(U32)
        v32 = v_hbm.bitcast(U32)

        def kcp(p):
            return pltpu.make_async_copy(k32.at[pl.ds(2 * p, 2), :, pl.ds(CP0, NCP)], kb.at[pl.ds(2 * p, 2)], ksem.at[p])

        def vcp(p):
            return pltpu.make_async_copy(v32.at[pl.ds(2 * p, 2), :, pl.ds(CP0, NCP)], vb.at[pl.ds(2 * p, 2)], vsem.at[p])

        wq_cp = pltpu.make_async_copy(wq_hbm.bitcast(U32), wqb, wsem.at[0])
        wo_cp = pltpu.make_async_copy(wo_hbm.bitcast(U32), wob, wsem.at[1])
        w3_cp = pltpu.make_async_copy(w3_hbm.bitcast(U32), w3b, wsem.at[2])
        x_cp = pltpu.make_async_copy(x_hbm, xbuf, wsem.at[3])
        o_cp = pltpu.make_async_copy(obuf, o_hbm, wsem.at[4])
        w4_cp = [pltpu.make_async_copy(w4_hbm.bitcast(U32).at[pl.ds(i * R4, R4)], w4b.at[pl.ds(i * R4, R4)], wsem.at[5 + i])
                 for i in range(W4C)]

        wq_cp.start()
        x_cp.start()
        kcp(0).start()
        wo_cp.start()
        for i in range(DEPTH):
            kcp(i + 1).start()
            vcp(i).start()

        low = lax.broadcasted_iota(jnp.int32, (8, 128), 0) < 4
        in_a = lax.broadcasted_iota(jnp.int32, (8, PD), 1) < DH

        def make_expand_matrix():
            row = lax.broadcasted_iota(jnp.int32, (128, 512), 0)
            col = lax.broadcasted_iota(jnp.int32, (128, 512), 1)
            hi = row >> 6
            jj = row & 63
            u = col >> 7
            cond = ((u >> 1) == hi) & ((col & 127) == ((jj >> 3) << 4) + ((u & 1) << 3) + (jj & 7))
            eca[...] = jnp.where(cond, 1.0, 0.0).astype(BF)

        def retile_wq():
            def body(g, _):
                for c in range(24):
                    a = wqb[g, 0, c]
                    b = wqb[g, 1, c]
                    wqb[g, 0, c] = jnp.where(low, a, pltpu.roll(b, 4, 0))
                    wqb[g, 1, c] = jnp.where(low, pltpu.roll(a, 4, 0), b)
                return _
            lax.fori_loop(0, 40, body, 0)

        def retile_wo():
            def body(gg, _):
                for u in range(4):
                    g = gg * 4 + u
                    raw = [wob[g, p] for p in range(5)]
                    rot = [pltpu.roll(r, 4, 0) for r in raw]
                    for c in range(5):
                        t1, t2 = c, 5 + c
                        top = raw[t1 // 2] if t1 % 2 == 0 else rot[t1 // 2]
                        bot = rot[t2 // 2] if t2 % 2 == 0 else raw[t2 // 2]
                        wob[g, c] = jnp.where(low, top, bot)
                return _
            lax.fori_loop(0, 96, body, 0)

        def transpose_v(p):
            def body(ci, _):
                c = NV + ci
                nat = [[], []]
                for hh in range(2):
                    raw = [vb[2 * p + hh, r, c] for r in range(24)]
                    for g in range(12):
                        a, b = raw[2 * g], raw[2 * g + 1]
                        nat[0].append(jnp.where(low, a, pltpu.roll(b, 4, 0)))
                        nat[1].append(jnp.where(low, pltpu.roll(a, 4, 0), b))
                outs = []
                for cc in range(2):
                    t = _u(_bf(jnp.concatenate(nat[cc], axis=0)).T)
                    for j in range(3):
                        for mm in range(8):
                            outs.append(t[mm * 8:(mm + 1) * 8, j * 128:(j + 1) * 128])
                for s, v in enumerate(outs):
                    vb[2 * p + s // 24, s % 24, c] = v
                return _
            lax.fori_loop(0, MC, body, 0)

        def widen_v(p):
            def body(hh, _):
                h = 2 * p + hh
                for c in range(PPK):
                    for r in range(24):
                        f = _bf(vb[h, r, c]).astype(F32)
                        vf[h, r, c, 0] = f[0:8]
                        vf[h, r, c, 1] = f[8:16]
                return _
            lax.fori_loop(0, 2, body, 0)

        def qproj(p):
            cols = []
            for u in range(3):
                t = 3 * p + u
                cols.append(_bf(wqb[:, t % 2, t // 2].reshape(320, 128)))
            return jnp.dot(xlb[...], jnp.concatenate(cols, axis=1), preferred_element_type=F32)

        def expand(q):
            q = (q * QSCALE).astype(BF)
            qs = jnp.concatenate([q[:, 0:128], q[:, 128:256], q[:, 256:384]], axis=0)
            ex = jnp.dot(qs, eca[...], preferred_element_type=F32)

            def tile(t, hi):
                return jnp.concatenate([ex[t * 8:(t + 1) * 8, (2 * hi) * 128:(2 * hi + 1) * 128],
                                        ex[t * 8:(t + 1) * 8, (2 * hi + 1) * 128:(2 * hi + 2) * 128]], axis=0)
            la = jnp.concatenate([tile(0, 0), tile(0, 1), tile(1, 0)], axis=1).astype(BF)
            lb_ = jnp.concatenate([tile(1, 1), tile(2, 0), tile(2, 1)], axis=1).astype(BF)
            return la, lb_

        def qk(h, L, dst, mxd, gates=None, z=None, qa=0, qb=0, cb=None):
            ms = []
            for c in range(NCP):
                w = kb[h, :, c]
                gi = -1 if gates is None else min(qa + ((qb - qa) * c) // NCP, len(gates) - 1)
                if gi >= 0:
                    fz = _u(gates[gi]) & z
                    w = jnp.concatenate([w[r] | fz if r == GR else w[r] for r in range(24)], axis=0)
                else:
                    w = w.reshape(192, 128)
                s = jnp.dot(L, _bf(w), preferred_element_type=F32)
                dst[:, c * 128:(c + 1) * 128] = s
                ms.append(s)
                if cb is not None and c == XK:
                    cb()
            m = ms[0]
            for t in ms[1:]:
                m = jnp.maximum(m, t)
            mxd[...] = jnp.maximum(m[0:8], m[8:16])

        def expo(src, mxs, edst):
            mh = jnp.broadcast_to(jnp.max(mxs[...], axis=1, keepdims=True), (8, 128))
            parts = []
            for c in range(NCP):
                e0 = jnp.exp2(src[0:8, c * 128:(c + 1) * 128] - mh)
                e1 = jnp.exp2(src[8:16, c * 128:(c + 1) * 128] - mh)
                edst[0:8, c * 128:(c + 1) * 128] = e0
                edst[8:16, c * 128:(c + 1) * 128] = e1
                parts.append(e1)
            return parts

        def pv_vpu(h, esrc, par, eparts, pre, z, prev):
            hist = list(prev) if prev is not None else []
            eg, egs = (EGE, EGSE) if par == 0 else (EG, EGS)
            outs = []
            l = jnp.zeros((8, 128), F32)
            for gi in range(NG):
                deps = []
                if len(hist) >= CD and not (par == 0 and gi < CD0):
                    deps.append(hist[-CD])
                if eg <= gi < eg + egs:
                    k0 = ((gi - eg) * NCP) // egs
                    k1 = ((gi - eg + 1) * NCP) // egs
                    for k in range(k0, k1):
                        if (k - k0) % ESK == ESK - 1 or k == k1 - 1:
                            deps.append(eparts[k])
                for pg, val in pre:
                    if pg == gi:
                        deps.append(val)
                if deps:
                    t = _u(deps[0])
                    for dd in deps[1:]:
                        t = t | _u(dd)
                    acc0 = pltpu.bitcast(t & z, F32)
                else:
                    acc0 = jnp.zeros((8, 128), F32)
                acc = [acc0 for _ in range(NA)]
                for c in range(NCP):
                    if c >= NV and gi != LGRP:
                        continue
                    e0 = esrc[0:8, c * 128:(c + 1) * 128]
                    e1 = esrc[8:16, c * 128:(c + 1) * 128]
                    if gi == LGRP:
                        l = l + (e0 + e1)
                    if c >= NV:
                        continue
                    for r in range(NA):
                        if c < PPK:
                            f0, f1 = vf[h, gi * NA + r, c, 0], vf[h, gi * NA + r, c, 1]
                        else:
                            f = _bf(vb[h, gi * NA + r, c]).astype(F32)
                            f0, f1 = f[0:8], f[8:16]
                        acc[r] = acc[r] + (f0 * e0 + f1 * e1)
                for r in range(NA):
                    r0 = par * DH + (gi * NA + r) * 8
                    accb[r0:r0 + 8, :] = acc[r]
                hist.append(acc[0])
                outs.append(acc[0])
            lb[par * 8:(par + 1) * 8, :] = l
            return outs

        def pv_mxu(p, e_even, e_odd, gates, z):
            lhs = []
            rhs = []
            for ci in range(MC):
                c = NV + ci
                for cc in range(2):
                    lhs.append(jnp.concatenate([e_even[cc * 8:(cc + 1) * 8, ci * 128:(ci + 1) * 128],
                                                e_odd[cc * 8:(cc + 1) * 8, c * 128:(c + 1) * 128]], axis=0))
                    fz = _u(gates[min(MA + ((MB - MA) * (2 * ci + cc)) // (2 * MC), len(gates) - 1)]) & z
                    cols = []
                    for j in range(3):
                        rows = []
                        for mm in range(8):
                            s = (cc * 3 + j) * 8 + mm
                            v = vb[2 * p + s // 24, s % 24, c]
                            rows.append(v | fz if (mm == 7 and j == 0) else v)
                        cols.append(jnp.concatenate(rows, axis=0))
                    rhs.append(jnp.concatenate(cols, axis=1))
            e = jnp.concatenate(lhs, axis=1).astype(BF)
            out = jnp.dot(e, _bf(jnp.concatenate(rhs, axis=0)), preferred_element_type=F32)
            return jnp.where(in_a, out[0:8], out[8:16])

        def finish():
            o = jnp.sum(accb[...].T, axis=0, keepdims=True)
            inv = 1.0 / jnp.sum(lb[...], axis=1, keepdims=True)
            return (o + omb[...]) * jnp.where(in_a, inv[0:8], inv[8:16])

        def wo_dot(o, p):
            g0 = pl.multiple_of(p * 24, 8)
            cols = [_bf(wob[pl.ds(g0, 24), c].reshape(192, 128)) for c in range(5)]
            return jnp.dot(o.astype(BF), jnp.concatenate(cols, axis=1), preferred_element_type=F32)

        def block(p):
            z = jnp.broadcast_to(lax.shift_right_arithmetic(p, 31), (8, 128)).astype(U32)
            p1 = jnp.minimum(p + 1, NP - 1)
            p2 = jnp.minimum(p + 2, NP - 1)
            le = Lb[p1 % 2, 0]
            lo = Lb[p1 % 2, 1]
            q = qproj(p2)

            def issue_expand():
                la, lb_ = expand(q)
                Lb[p2 % 2, 0] = la
                Lb[p2 % 2, 1] = lb_
            o = finish()
            ge = pv_vpu(2 * p, ea, 0, expo(sa, mxa, eb), [(FG, o[:, 0:128])], z, None)
            qk(2 * p1, le, sb, mxb, ge, z, QAE, QBE, issue_expand)
            xab[...] += wo_dot(o, jnp.maximum(p - 1, 0))
            e_even = ea[:, NV * 128:NCP * 128]
            go = pv_vpu(2 * p + 1, eb, 1, expo(sb, mxb, ea), [], z, ge)
            qk(2 * p1 + 1, lo, sa, mxa, ge + go, z, QA, QB)
            omb[...] = pv_mxu(p, e_even, eb, ge + go, z)

        def attention(x, first):
            xlb[...] = _ln(x).astype(BF)
            if first:
                make_expand_matrix()
                wq_cp.wait()
                retile_wq()
            q0 = qproj(0)
            q1 = qproj(1)
            la, lb_ = expand(q0)
            la1, lb1 = expand(q1)
            Lb[1, 0] = la1
            Lb[1, 1] = lb1
            if first:
                kcp(0).wait()
            qk(0, la, sb, mxb)
            qk(1, lb_, sa, mxa)
            expo(sb, mxb, ea)
            xab[...] = jnp.zeros_like(xab)
            accb[...] = jnp.zeros_like(accb)
            lb[...] = jnp.ones_like(lb)
            omb[...] = jnp.zeros_like(omb)
            if first:
                wo_cp.wait()
                retile_wo()

            def body(p, carry):
                if first:
                    @pl.when(p + 1 < NP)
                    def _():
                        kcp(p + 1).wait()
                    vcp(p).wait()

                    @pl.when(p + DEPTH < NP)
                    def _():
                        i = p + DEPTH

                        @pl.when(i + 1 < NP)
                        def _():
                            kcp(i + 1).start()
                        vcp(i).start()

                        @pl.when(i == NP - 1)
                        def _():
                            w3_cp.start()
                            for c in w4_cp:
                                c.start()

                    transpose_v(p)
                    if PPK:
                        widen_v(p)
                block(p)
                return carry

            lax.fori_loop(0, NP, body, 0)
            return x + xab[...] + wo_dot(finish(), NP - 1)

        def mlp(x, first):
            u, h = _ln_ln(x)
            if first:
                w3_cp.wait()
            g = jnp.dot(h.astype(BF), _bf(w3b[...]), preferred_element_type=F32)
            g = jax.nn.gelu(g, approximate=True).astype(BF)
            y = x + u
            if first:
                for i in range(W4C):
                    w4_cp[i].wait()
                    y = y + jnp.dot(g[:, i * 2 * R4:(i + 1) * 2 * R4], _bf(w4b[i * R4:(i + 1) * R4, :]),
                                    preferred_element_type=F32)
            else:
                y = y + jnp.dot(g, _bf(w4b[...]), preferred_element_type=F32)
            return y

        x_cp.wait()
        x = jnp.broadcast_to(xbuf[0].astype(F32), (8, D))
        x = attention(x, True)
        x = mlp(x, True)
        x = attention(x, False)
        x = mlp(x, False)
        obuf[0] = x[0:1].astype(BF)
        o_cp.start()
        o_cp.wait()

    def fn(A_x, A_k_cache, A_v_cache, A_wq, A_wo, B_x, B_w1, B_w2, B_w3, B_w4):
        kT = _raw2(jnp.swapaxes(A_k_cache[0], 1, 2))
        vT = _raw2(jnp.swapaxes(A_v_cache[0], 1, 2))
        S = pltpu.VMEM((16, W // 2), F32)
        M = pltpu.VMEM((8, 128), F32)
        return pl.pallas_call(
            kernel,
            out_shape=jax.ShapeDtypeStruct((1, 1, D), BF),
            in_specs=[pl.BlockSpec(memory_space=pl.ANY)] * 7,
            out_specs=pl.BlockSpec(memory_space=pl.ANY),
            scratch_shapes=[
                pltpu.VMEM((H, 24, NCP, 8, 128), U32),
                pltpu.VMEM((H, 24, NCP, 8, 128), U32),
                pltpu.VMEM((H, 24, max(PPK, 1), 2, 8, 128), F32),
                pltpu.VMEM((40, 2, 24, 8, 128), U32),
                pltpu.VMEM((384, 5, 8, 128), U32),
                pltpu.VMEM((D // 2, F), U32),
                pltpu.VMEM((F // 2, D), U32),
                pltpu.VMEM((128, 512), BF),
                S, S, S, S, M, M,
                pltpu.VMEM((PD, 128), F32),
                pltpu.VMEM((16, 128), F32),
                pltpu.VMEM((2, 2, 16, PD), BF),
                pltpu.VMEM((8, D), F32),
                pltpu.VMEM((8, PD), F32),
                pltpu.VMEM((8, D), BF),
                pltpu.VMEM((1, 1, D), BF),
                pltpu.VMEM((1, 1, D), BF),
                pltpu.SemaphoreType.DMA((NP,)),
                pltpu.SemaphoreType.DMA((NP,)),
                pltpu.SemaphoreType.DMA((5 + W4C,)),
            ],
            compiler_params=pltpu.CompilerParams(vmem_limit_bytes=127 * 2**20, disable_semaphore_checks=True),
        )(A_x, kT, vT, _raw2(A_wq).reshape(40, 2, 24, 16, 128), _raw5(A_wo), B_w3, B_w4)
    return fn


@jax.jit
def pallas_interleave_layers__sliding_block_cached__mixer_s_mlp__decode_kernel(
    A_x: jax.Array,
    A_k_cache: jax.Array,
    A_v_cache: jax.Array,
    A_wq: jax.Array,
    A_wo: jax.Array,
    B_x: jax.Array,
    B_w1: jax.Array,
    B_w2: jax.Array,
    B_w3: jax.Array,
    B_w4: jax.Array,
):
    sk = A_k_cache.shape[2]
    w = min(4096, max(256, sk // 4))
    return build(sk, w)(A_x, A_k_cache, A_v_cache, A_wq, A_wo, B_x, B_w1, B_w2, B_w3, B_w4)
```
